```python
import jax
import jax.numpy as jnp

def _softmax(x, axis=-1):
    return jax.nn.softmax(x, axis=axis)
def _gelu(x):
    return jax.nn.gelu(x, approximate=True)
def _silu(x):
    return jax.nn.silu(x)
def _sigmoid(x):
    return jax.nn.sigmoid(x)
def _layernorm(x, axis=-1, eps=1e-5):
    m = jnp.mean(x, axis=axis, keepdims=True)
    v = jnp.var(x, axis=axis, keepdims=True)
    return (x - m) / jnp.sqrt(v + eps)
def _scatter_add(tgt, idx, src, axis=0):
    return tgt.at[idx].add(src)
def _segment_sum(src, seg, n):
    return jax.ops.segment_sum(src, seg, n)
class _Rng:
    def __init__(self, key):
        self._k = key
    def _next(self):
        self._k, sub = jax.random.split(self._k)
        return sub
    def normal(self, shape):
        return jax.random.normal(self._next(), shape, dtype=jnp.bfloat16)
    def randint(self, lo, hi, shape):
        return jax.random.randint(self._next(), shape, lo, hi, dtype=jnp.int32)
    def uniform(self, shape, lo=0.0, hi=1.0):
        return jax.random.uniform(self._next(), shape, jnp.bfloat16, lo, hi)
    def permutation(self, n):
        return jax.random.permutation(self._next(), n)


kernel_name = 'interleave_layers__ssm_conv_s5__ssm_conv_h3__prompt'

def setup_inputs():
    _rng = _Rng(jax.random.key(int.from_bytes(__import__("os").urandom(4), "little")))
    _w = (lambda a: (lambda t: t.astype(jnp.bfloat16) if jnp.issubdtype(t.dtype, jnp.floating) else t)(jnp.asarray(a)))
    def _A_setup():
        B, S, D = 1, 2048, 640
        P = D
        Lambda_re = -0.5 * jnp.exp((lambda *s: _rng.normal(s) * 0.05)(P))
        Lambda_im = (lambda *s: _rng.normal(s) * 0.05)(P) * 1.0
        B_re = (lambda *s: _rng.normal(s) * 0.05)(P, D) * (D ** -0.5)
        B_im = (lambda *s: _rng.normal(s) * 0.05)(P, D) * (D ** -0.5)
        C_re = (lambda *s: _rng.normal(s) * 0.05)(D, P) * (P ** -0.5)
        C_im = (lambda *s: _rng.normal(s) * 0.05)(D, P) * (P ** -0.5)
        log_dt = (lambda *s: _rng.normal(s) * 0.05)(P) * 0.3 - 2.0
        Dskip = (lambda *s: _rng.normal(s) * 0.05)(D)
        return {
            "x": _w((lambda *s: _rng.normal(s) * 0.05)(B, S, D)),
            "Lambda_re": _w(Lambda_re),
            "Lambda_im": _w(Lambda_im),
            "B_re": _w(B_re),
            "B_im": _w(B_im),
            "C_re": _w(C_re),
            "C_im": _w(C_im),
            "log_dt": _w(log_dt),
            "Dskip": _w(Dskip),
        }
    _A_in = _A_setup()

    def _B_setup():
        B, S, D = 1, 2048, 640
        ks = 4
        return {
            "q": _w((lambda *s: _rng.normal(s) * 0.05)(B, S, D)),
            "k": _w((lambda *s: _rng.normal(s) * 0.05)(B, S, D)),
            "v": _w((lambda *s: _rng.normal(s) * 0.05)(B, S, D)),
            "shift_k": _w((lambda *s: _rng.normal(s) * 0.05)(D, ks) * 0.5),
            "ssm_k": _w((lambda *s: _rng.normal(s) * 0.05)(D, S) * (1.0 / S ** 0.5)),
            "ssm_D": _w((lambda *s: _rng.normal(s) * 0.05)(D)),
        }
    _B_in = _B_setup()

    return {
        "A_x": _A_in["x"],
        "A_Lambda_re": _A_in["Lambda_re"],
        "A_Lambda_im": _A_in["Lambda_im"],
        "A_B_re": _A_in["B_re"],
        "A_B_im": _A_in["B_im"],
        "A_C_re": _A_in["C_re"],
        "A_C_im": _A_in["C_im"],
        "A_log_dt": _A_in["log_dt"],
        "A_Dskip": _A_in["Dskip"],
        "B_q": _B_in["q"],
        "B_k": _B_in["k"],
        "B_v": _B_in["v"],
        "B_shift_k": _B_in["shift_k"],
        "B_ssm_k": _B_in["ssm_k"],
        "B_ssm_D": _B_in["ssm_D"],
    }

def reference(A_x, A_Lambda_re, A_Lambda_im, A_B_re, A_B_im, A_C_re, A_C_im, A_log_dt, A_Dskip, B_q, B_k, B_v, B_shift_k, B_ssm_k, B_ssm_D):
    def _A_ref(x, Lambda_re, Lambda_im, B_re, B_im, C_re, C_im, log_dt, Dskip):
        Bsz, L, H = x.shape
        Lam = Lambda_re + 1j * Lambda_im
        Bmat = B_re + 1j * B_im
        Cmat = C_re + 1j * C_im
        dt = jnp.exp(log_dt)
        Lam_bar = jnp.exp(dt * Lam)
        B_bar = ((Lam_bar - 1.0) / Lam)[:, None] * Bmat
        Bu = jnp.einsum("bld,pd->blp", x + 0j, B_bar)
        h = jnp.zeros_like(Bu[:, 0, :])
        hs = []
        for t in range(L):
            h = Lam_bar[None, :] * h + Bu[:, t, :]
            hs.append(h)
        hseq = jnp.stack(hs, 1)
        y = 2.0 * jnp.einsum("blp,dp->bld", hseq, Cmat).real + x * Dskip[None, None, :]
        return y

    def _B_ref(q, k, v, shift_k, ssm_k, ssm_D):
        B, S, D = q.shape
        ks = shift_k.shape[-1]
        k_pad = jnp.pad(k, ((0, 0), (ks - 1, 0), (0, 0)))
        k_shift = jnp.zeros_like(k)
        for t in range(ks):
            k_shift = k_shift + k_pad[:, t:t + S, :] * shift_k[:, ks - 1 - t][None, None, :]
        kv = k_shift * v
        L = 2 * S
        kv_pad = jnp.pad(kv, ((0, 0), (0, S), (0, 0)))
        kf_pad = jnp.pad(ssm_k, ((0, 0), (0, S)))
        kv_f = (lambda x, axes=(-2,-1): jnp.fft.rfft2(x.astype(jnp.float32), axes=axes))(kv_pad[:, None, :, :], axes=(1, 2))
        kf_f = (lambda x, axes=(-2,-1): jnp.fft.rfft2(x.astype(jnp.float32), axes=axes))(kf_pad[:, None, :], axes=(1, 2))
        kf_f = (lambda x, *d: x.transpose(*d))(kf_f, 1, 2, 0)
        y_f = kv_f * kf_f[None, :, :, :]
        y = (lambda x, s, axes=(-2,-1): jnp.fft.irfft2(x, s=s, axes=axes).astype(jnp.bfloat16))(y_f, (1, L), axes=(1, 2))[:, 0, :S, :]
        y = y + kv * ssm_D[None, None, :]
        return q * y

    x = A_x
    x = x + _A_ref(_layernorm(x, axis=-1), A_Lambda_re, A_Lambda_im, A_B_re, A_B_im, A_C_re, A_C_im, A_log_dt, A_Dskip)
    x = x + _B_ref(_layernorm(x, axis=-1), B_k, B_v, B_shift_k, B_ssm_k, B_ssm_D)
    x = x + _A_ref(_layernorm(x, axis=-1), A_Lambda_re, A_Lambda_im, A_B_re, A_B_im, A_C_re, A_C_im, A_log_dt, A_Dskip)
    x = x + _B_ref(_layernorm(x, axis=-1), B_k, B_v, B_shift_k, B_ssm_k, B_ssm_D)
    return x
```

```python
import functools
import numpy as np
import jax
import jax.numpy as jnp
from jax import lax
import jax.experimental.pallas as pl
import jax.experimental.pallas.tpu as pltpu

S = 2048
D = 640
L = 128
NCH = S // L
NT = D // 128
F32 = jnp.float32
BF16 = jnp.bfloat16


def _dft_consts():
    n = 2 * L
    ks = np.concatenate([np.arange(0, L, 2), np.arange(1, L, 2)])
    t = np.arange(L)
    th = 2.0 * np.pi * np.outer(ks + 0.5, t) / n
    c = np.cos(th)
    s = -np.sin(th)
    f = np.concatenate([c.reshape(L // 8, 8, L), s.reshape(L // 8, 8, L)], axis=1)
    f = f.reshape(2 * L, L)
    g = f.T / L
    return f.astype(np.float32), np.ascontiguousarray(g).astype(np.float32)


_F_NP, _G_NP = _dft_consts()


def _ln_rows(x):
    m = jnp.sum(x, axis=-1, keepdims=True) * (1.0 / D)
    xc = x - m
    v = jnp.sum(xc * xc, axis=-1, keepdims=True) * (1.0 / D)
    return xc * lax.rsqrt(v + 1e-5)


def _scan_block(bu_re, bu_im, tabs, carry, rows):
    nj = rows // 8
    h_re = [[None] * nj for _ in range(NT)]
    h_im = [[None] * nj for _ in range(NT)]
    carry = list(carry)
    for j in range(nj):
        for n in range(NT):
            pr = bu_re[n][8 * j:8 * j + 8]
            pi = bu_im[n][8 * j:8 * j + 8]
            for si, sh in enumerate((1, 2, 4)):
                mr = tabs(2 * si, n)
                mi = tabs(2 * si + 1, n)
                sr = pltpu.roll(pr, sh, 0)
                s_i = pltpu.roll(pi, sh, 0)
                pr, pi = pr + (mr * sr - mi * s_i), pi + (mr * s_i + mi * sr)
            cr, ci = carry[n]
            wr = tabs(6, n)
            wi = tabs(7, n)
            hr = pr + (wr * cr - wi * ci)
            hi = pi + (wr * ci + wi * cr)
            h_re[n][j] = hr
            h_im[n][j] = hi
            carry[n] = (jnp.broadcast_to(hr[7:8], (8, 128)), jnp.broadcast_to(hi[7:8], (8, 128)))
    h_re = [jnp.concatenate(l, axis=0) for l in h_re]
    h_im = [jnp.concatenate(l, axis=0) for l in h_im]
    return h_re, h_im, carry


def _kernel(x_ref, lre_ref, lim_ref, bre_ref, bim_ref, cre_ref, cim_ref, ldt_ref, dsk_ref,
            k_ref, v_ref, shk_ref, ssmk_ref, ssmd_ref, f_ref, g_ref,
            o_ref,
            bb_ref, tab_ref, kf_ref, u_ref, kp_ref, z_ref, yk_ref, x1_ref,
            *, T):
    lre = lre_ref[...].astype(F32)
    lim = lim_ref[...].astype(F32)
    dt = jnp.exp(ldt_ref[...].astype(F32)).astype(BF16).astype(F32)
    a = dt * lre
    b = dt * lim
    row = lax.broadcasted_iota(jnp.int32, (8, D), 0)
    for si, sh in enumerate((1, 2, 4)):
        e = jnp.exp(a * float(sh))
        cr = jnp.broadcast_to(e * jnp.cos(b * float(sh)), (8, D))
        ci = jnp.broadcast_to(-e * jnp.sin(b * float(sh)), (8, D))
        tab_ref[2 * si] = jnp.where(row >= sh, cr, 0.0)
        tab_ref[2 * si + 1] = jnp.where(row >= sh, ci, 0.0)
    nn = (row + 1).astype(F32)
    e = jnp.exp(a * nn)
    tab_ref[6] = e * jnp.cos(b * nn)
    tab_ref[7] = -e * jnp.sin(b * nn)
    e1 = jnp.exp(a)
    lr = e1 * jnp.cos(b) - 1.0
    li = e1 * jnp.sin(b)
    den = lre * lre + lim * lim
    cfr = 2.0 * (lr * lre + li * lim) / den
    cfi = 2.0 * (li * lre - lr * lim) / den
    cfr_c = jnp.transpose(jnp.broadcast_to(cfr, (128, D)))
    cfi_c = jnp.transpose(jnp.broadcast_to(cfi, (128, D)))
    for n in range(NT):
        br = bre_ref[:, 128 * n:128 * n + 128].astype(F32)
        bi = bim_ref[:, 128 * n:128 * n + 128].astype(F32)
        bb_ref[0:D, 128 * n:128 * n + 128] = (cfr_c * br - cfi_c * bi).astype(BF16)
        bb_ref[D:2 * D, 128 * n:128 * n + 128] = (-(cfr_c * bi + cfi_c * br)).astype(BF16)

    shk = jnp.transpose(shk_ref[...].astype(F32))
    ssmd = ssmd_ref[...].astype(F32)
    dsk = dsk_ref[...].astype(F32)

    for n in range(NT):
        kf_ref[n, 0:8, :] = jnp.zeros((8, 128), F32)

    def p0_body(c, kprev):
        r0 = pl.multiple_of(c * L, L)
        kblk = k_ref[pl.ds(r0, L), :].astype(F32)
        for n in range(NT):
            kf_ref[n, pl.ds(r0 + 8, L), :] = kblk[:, 128 * n:128 * n + 128]
        vblk = v_ref[pl.ds(r0, L), :].astype(F32)
        kvs = []
        for n in range(NT):
            acc = kblk[:, 128 * n:128 * n + 128] * shk[0:1, 128 * n:128 * n + 128]
            for i in range(1, 4):
                acc = acc + kf_ref[n, pl.ds(r0 + 8 - i, L), :] * shk[i:i + 1, 128 * n:128 * n + 128]
            kvs.append(acc * vblk[:, 128 * n:128 * n + 128])
        kv = jnp.concatenate(kvs, axis=1).astype(BF16)
        yk_ref[pl.ds(r0, L), :] = (kv.astype(F32) * ssmd).astype(BF16)
        fm = f_ref[...]
        u_ref[c] = jnp.dot(fm, kv, preferred_element_type=F32)
        kc = lax.dot_general(fm, ssmk_ref[:, pl.ds(r0, L)], (((1,), (1,)), ((), ())),
                             preferred_element_type=F32)
        kp = kprev
        outs = []
        for j in range(16):
            sgn = 1.0 if j < 8 else -1.0
            re = kc[16 * j:16 * j + 8]
            im = kc[16 * j + 8:16 * j + 16]
            pre = kp[16 * j:16 * j + 8]
            pim = kp[16 * j + 8:16 * j + 16]
            if sgn > 0:
                outs += [re - pim, im + pre]
            else:
                outs += [re + pim, im - pre]
        kp_ref[c] = jnp.concatenate(outs, axis=0)
        return kc

    lax.fori_loop(0, NCH, p0_body, jnp.zeros((2 * L, D), F32))

    def tabs(i, n):
        return tab_ref[i, :, 128 * n:128 * n + 128]

    def s5_block(xn, carry):
        bu = lax.dot_general(xn.astype(BF16), bb_ref[...], (((1,), (1,)), ((), ())),
                             preferred_element_type=F32)
        bu_re = [bu[:, 128 * n:128 * n + 128] for n in range(NT)]
        bu_im = [bu[:, D + 128 * n:D + 128 * n + 128] for n in range(NT)]
        h_re, h_im, carry = _scan_block(bu_re, bu_im, tabs, carry, T)
        hr = jnp.concatenate(h_re, axis=1).astype(BF16)
        hi = jnp.concatenate(h_im, axis=1).astype(BF16)
        y = lax.dot_general(hr, cre_ref[...], (((1,), (1,)), ((), ())), preferred_element_type=F32)
        y = y + lax.dot_general(hi, cim_ref[...], (((1,), (1,)), ((), ())), preferred_element_type=F32)
        return y, carry

    zero_carry = [(jnp.zeros((8, 128), F32), jnp.zeros((8, 128), F32)) for _ in range(NT)]

    nblk = S // T
    fper = NCH // nblk

    def interchunk(g):
        r = pl.multiple_of(g * 16, 16)
        for n in range(NT):
            sl = slice(128 * n, 128 * n + 128)
            for a_ in range(NCH):
                zr = None
                zi = None
                for b_ in range(a_ + 1):
                    kr = kp_ref[a_ - b_, pl.ds(r, 8), sl]
                    ki = kp_ref[a_ - b_, pl.ds(r + 8, 8), sl]
                    ur = u_ref[b_, pl.ds(r, 8), sl]
                    ui = u_ref[b_, pl.ds(r + 8, 8), sl]
                    tr = kr * ur - ki * ui
                    ti = kr * ui + ki * ur
                    zr = tr if zr is None else zr + tr
                    zi = ti if zi is None else zi + ti
                z_ref[a_, pl.ds(r, 16), sl] = jnp.concatenate([zr, zi], axis=0).astype(BF16)

    def p1_body(j, carry):
        r0 = pl.multiple_of(j * T, T)
        x = x_ref[pl.ds(r0, T), :].astype(F32)
        xn = _ln_rows(x)
        y, carry = s5_block(xn, carry)
        x1_ref[pl.ds(r0, T), :] = x + y + xn * dsk
        for f in range(fper):
            interchunk(j * fper + f)
        return carry

    lax.fori_loop(0, nblk, p1_body, zero_carry)

    cper = T // L

    def p2_body(j, carry):
        r0 = pl.multiple_of(j * T, T)
        ys = []
        for c in range(cper):
            yc = jnp.dot(g_ref[...], z_ref[j * cper + c], preferred_element_type=F32)
            ys.append(yc)
        yconv = ys[0] if cper == 1 else jnp.concatenate(ys, axis=0)
        yy = (yconv.astype(BF16).astype(F32) + yk_ref[pl.ds(r0, T), :].astype(F32)).astype(BF16).astype(F32)
        x1 = x1_ref[pl.ds(r0, T), :]
        x2 = x1 + _ln_rows(x1) * yy
        xn = _ln_rows(x2)
        y, carry = s5_block(xn, carry)
        x3 = x2 + y + xn * dsk
        o_ref[pl.ds(r0, T), :] = x3 + _ln_rows(x3) * yy
        return carry

    lax.fori_loop(0, nblk, p2_body, zero_carry)


def make(T=128):
    @jax.jit
    def fn(A_x, A_Lambda_re, A_Lambda_im, A_B_re, A_B_im, A_C_re, A_C_im, A_log_dt, A_Dskip,
           B_q, B_k, B_v, B_shift_k, B_ssm_k, B_ssm_D):
        del B_q
        row = lambda t: t.reshape(1, D)
        args = (A_x.reshape(S, D), row(A_Lambda_re), row(A_Lambda_im), A_B_re, A_B_im, A_C_re, A_C_im,
                row(A_log_dt), row(A_Dskip), B_k.reshape(S, D), B_v.reshape(S, D), B_shift_k, B_ssm_k,
                row(B_ssm_D), jnp.asarray(_F_NP, BF16), jnp.asarray(_G_NP, BF16))
        out = pl.pallas_call(
            functools.partial(_kernel, T=T),
            out_shape=jax.ShapeDtypeStruct((S, D), F32),
            scratch_shapes=[
                pltpu.VMEM((2 * D, D), BF16),
                pltpu.VMEM((8, 8, D), F32),
                pltpu.VMEM((NT, S + 8, 128), F32),
                pltpu.VMEM((NCH, 2 * L, D), F32),
                pltpu.VMEM((NCH, 2 * L, D), F32),
                pltpu.VMEM((NCH, 2 * L, D), BF16),
                pltpu.VMEM((S, D), BF16),
                pltpu.VMEM((S, D), F32),
            ],
            compiler_params=pltpu.CompilerParams(vmem_limit_bytes=100 * 1024 * 1024),
            name="ssm_fused",
        )(*args)
        return out.reshape(1, S, D)
    return fn


pallas_interleave_layers__ssm_conv_s5__ssm_conv_h3__prompt_kernel = make(256)
```

```python
import functools
import numpy as np
import jax
import jax.numpy as jnp
from jax import lax
import jax.experimental.pallas as pl
import jax.experimental.pallas.tpu as pltpu

S = 2048
D = 640
L = 128
NCH = S // L
NT = D // 128
T = 256
NB = S // T
F32 = jnp.float32
BF16 = jnp.bfloat16
U32 = jnp.uint32
NZ = 1024


def _perm(np_):
    gsz = 8 * np_
    t = np.zeros(L, np.int64)
    for rho in range(L):
        g, r = divmod(rho, gsz)
        p, s = divmod(r, 8)
        t[rho] = gsz * g + np_ * s + p
    return t


def _dft_consts(np_):
    n = 2 * L
    ks = np.concatenate([np.arange(0, L, 2), np.arange(1, L, 2)])
    t = np.arange(L)
    th = 2.0 * np.pi * np.outer(ks + 0.5, t) / n
    c = np.cos(th)
    s = -np.sin(th)
    f = np.concatenate([c.reshape(L // 8, 8, L), s.reshape(L // 8, 8, L)], axis=1).reshape(2 * L, L)
    g = f.T / L
    p = _perm(np_)
    fp = f[:, p]
    gp = g[p, :]
    return (f.astype(np.float32), np.ascontiguousarray(fp).astype(np.float32),
            np.ascontiguousarray(gp).astype(np.float32))


def _ln_tiles(xs):
    s = xs[0]
    for x in xs[1:]:
        s = s + x
    m = jnp.sum(s, axis=-1, keepdims=True) * (1.0 / D)
    xc = [x - m for x in xs]
    q = xc[0] * xc[0]
    for x in xc[1:]:
        q = q + x * x
    v = jnp.sum(q, axis=-1, keepdims=True) * (1.0 / D)
    r = lax.rsqrt(v + 1e-5)
    return [x * r for x in xc]


def _cmac(br, bi, mr, mi, xr, xi):
    return br + (mr * xr - mi * xi), bi + (mr * xi + mi * xr)


def _scan_tile(bur, bui, tabf, carry, np_):
    gsz = 8 * np_
    row0 = lax.broadcasted_iota(jnp.int32, (8, 128), 0) == 0
    cr, ci = carry
    outr, outi = [], []
    for g in range(T // gsz):
        tab = tabf()
        lr, li = tab(8), tab(9)
        br = [bur[gsz * g + 8 * p:gsz * g + 8 * p + 8] for p in range(np_)]
        bi = [bui[gsz * g + 8 * p:gsz * g + 8 * p + 8] for p in range(np_)]
        vr, vi = br[0], bi[0]
        for p in range(1, np_):
            vr, vi = _cmac(br[p], bi[p], lr, li, vr, vi)
        for si, sh in enumerate((1, 2, 4)):
            vr, vi = _cmac(vr, vi, tab(2 * si), tab(2 * si + 1), pltpu.roll(vr, sh, 0), pltpu.roll(vi, sh, 0))
        hr, hi = _cmac(vr, vi, tab(6), tab(7), cr, ci)
        pr = jnp.where(row0, cr, pltpu.roll(hr, 1, 0))
        pi = jnp.where(row0, ci, pltpu.roll(hi, 1, 0))
        for p in range(np_ - 1):
            pr, pi = _cmac(br[p], bi[p], lr, li, pr, pi)
            outr.append(pr)
            outi.append(pi)
        outr.append(hr)
        outi.append(hi)
        cr = jnp.broadcast_to(hr[7:8], (8, 128))
        ci = jnp.broadcast_to(hi[7:8], (8, 128))
    return jnp.concatenate(outr, axis=0), jnp.concatenate(outi, axis=0), (cr, ci)


_NT_DIMS = (((1,), (1,)), ((), ()))


def _kernel(x_hbm, lre_ref, lim_ref, bre_hbm, bim_hbm, cre_hbm, cim_hbm, ldt_ref, dsk_ref,
            k_hbm, v_hbm, shk_in, ssmk_hbm, ssmd_ref, fn_ref, fp_ref, gp_ref, zero_ref,
            o_hbm,
            kb, vb, xb, sk, brb, bib, crb, cib, bb, tab_ref, u_ref, kk_ref, yp_ref, z_ref, yk_ref,
            xr_ref, ob, sems, osems, *, NP, opts):
    GS = 8 * NP
    HW = NP // 2
    NQ = 4
    RQ = S // NQ
    CQ = NCH // NQ
    util = opts.get("util", 0.8)

    copies = {}
    idx = [0]

    def add(name, src, dst):
        if opts.get("noin"):
            copies.setdefault(name, [])
            return
        c = pltpu.make_async_copy(src, dst, sems.at[idx[0]])
        idx[0] += 1
        copies.setdefault(name, []).append(c)
        c.start()

    def wait(name):
        for c in copies.pop(name):
            c.wait()

    def dma_kv(q):
        for c in range(q * CQ, (q + 1) * CQ):
            add(("kv", q), ssmk_hbm.at[:, pl.ds(L * c, L)], sk.at[c])
        for n in range(NT):
            add(("kv", q), k_hbm.at[pl.ds(RQ * q, RQ), pl.ds(128 * n, 128)], kb.at[n, pl.ds(16 + RQ * q, RQ)])
        for n in range(NT):
            add(("kv", q), v_hbm.at[pl.ds(RQ * q, RQ), pl.ds(128 * n, 128)], vb.at[n, pl.ds(RQ * q, RQ)])

    def dma_x(q):
        for n in range(NT):
            add(("x", q), x_hbm.at[pl.ds(RQ * q, RQ), pl.ds(128 * n, 128)], xb.at[n, pl.ds(RQ * q, RQ)])

    kb[:, 0:16, :] = jnp.zeros((NT, 16, 128), BF16)
    order = opts.get("order", "p0first")
    if order == "p0first":
        for q in range(NQ):
            dma_kv(q)
    for n in range(NT):
        add("b", bre_hbm.at[:, pl.ds(128 * n, 128)], brb.at[n])
        add("b", bim_hbm.at[:, pl.ds(128 * n, 128)], bib.at[n])
    dma_x(0)
    for n in range(NT):
        add("c", cre_hbm.at[:, pl.ds(128 * n, 128)], crb.at[n])
        add("c", cim_hbm.at[:, pl.ds(128 * n, 128)], cib.at[n])
    for q in range(NQ):
        if order != "p0first":
            dma_kv(q)
        if q > 0:
            dma_x(q)

    lre = lre_ref[...].astype(F32).reshape(1, D)
    lim = lim_ref[...].astype(F32).reshape(1, D)
    dt = jnp.exp(ldt_ref[...].astype(F32).reshape(1, D)).astype(BF16).astype(F32)
    a = dt * lre
    b = dt * lim
    row = lax.broadcasted_iota(jnp.int32, (8, D), 0)
    for si, sh in enumerate((1, 2, 4)):
        e = jnp.exp(a * float(sh * NP))
        cr = jnp.broadcast_to(e * jnp.cos(b * float(sh * NP)), (8, D))
        ci = jnp.broadcast_to(-e * jnp.sin(b * float(sh * NP)), (8, D))
        tab_ref[2 * si] = jnp.where(row >= sh, cr, 0.0)
        tab_ref[2 * si + 1] = jnp.where(row >= sh, ci, 0.0)
    nn = ((row + 1) * NP).astype(F32)
    e = jnp.exp(a * nn)
    tab_ref[6] = e * jnp.cos(b * nn)
    tab_ref[7] = -e * jnp.sin(b * nn)
    e1 = jnp.exp(a)
    l1r = e1 * jnp.cos(b)
    l1i = e1 * jnp.sin(b)
    tab_ref[8] = jnp.broadcast_to(l1r, (8, D))
    tab_ref[9] = jnp.broadcast_to(-l1i, (8, D))
    lr = l1r - 1.0
    den = lre * lre + lim * lim
    cfr = 2.0 * (lr * lre + l1i * lim) / den
    cfi = 2.0 * (l1i * lre - lr * lim) / den
    cfr_c = jnp.transpose(jnp.broadcast_to(cfr, (128, D)))
    cfi_c = jnp.transpose(jnp.broadcast_to(cfi, (128, D)))
    tab_ref[10] = jnp.broadcast_to(dsk_ref[...].astype(F32).reshape(1, D), (8, D))
    tab_ref[11] = jnp.broadcast_to(ssmd_ref[...].astype(F32).reshape(1, D), (8, D))
    shk = shk_in[...].astype(F32)
    for i in range(4):
        tab_ref[12 + i] = jnp.broadcast_to(shk[i:i + 1, :], (8, D))

    def tile(v, n):
        return v[:, 128 * n:128 * n + 128]

    kw = kb.bitcast(U32)
    vw = vb.bitcast(U32)
    xw = xb.bitcast(U32)
    bbw = bb.bitcast(U32)
    crw = crb.bitcast(U32)
    ciw = cib.bitcast(U32)
    zw = z_ref.bitcast(U32)
    skw = sk.bitcast(U32)
    never = zero_ref[0:8, :] != 0
    def tabv():
        z = 0
        return lambda i, n: tab_ref[z + i, :, 128 * n:128 * n + 128]

    def ldbf(w):
        return pltpu.bitcast(w, BF16)

    def tie(val, tick):
        if tick is None or not opts.get("ties", True):
            return val
        return jnp.where(never, tick, val)

    def unpack2(w):
        lo = pltpu.unpack_elementwise(w, index=0, packed_dtype=BF16, unpacked_dtype=F32)
        hi = pltpu.unpack_elementwise(w, index=1, packed_dtype=BF16, unpacked_dtype=F32)
        return lo, hi

    def bprep():
        wait("b")
        for k in range(NT):
            br = brb[k].astype(F32)
            bi = bib[k].astype(F32)
            re = (cfr_c * br - cfi_c * bi).astype(BF16)
            im = (-(cfr_c * bi + cfi_c * br)).astype(BF16)
            for n in range(NT):
                bb[n, k, 0:128, :] = re[128 * n:128 * n + 128]
                bb[n, k, 128:256, :] = im[128 * n:128 * n + 128]

    def kv_lumps(c, out):
        lumps = []
        for n in range(NT):
            for g in range(L // GS):
                def run(tick, n=n, g=g):
                    tb = tabv()
                    w0 = c * (L // 2) + g * GS // 2
                    cur, prev, vv = [], [], []
                    for q in range(HW):
                        w = kw[n, pl.ds(8 + w0 + q, 8, stride=HW), :]
                        cur += list(unpack2(w))
                        prev += list(unpack2(kw[n, pl.ds(8 + w0 - HW + q, 8, stride=HW), :]))
                        vv += list(unpack2(vw[n, pl.ds(w0 + q, 8, stride=HW), :]))
                    vv = [tie(x, tick) for x in vv[:1]] + vv[1:]
                    rows_ = []
                    for p in range(NP):
                        acc = None
                        for i in range(4):
                            src = cur[p - i] if p - i >= 0 else prev[NP + p - i]
                            t = src * tb(12 + i, n)
                            acc = t if acc is None else acc + t
                        rows_.append(acc * vv[p])
                    blk = jnp.concatenate(rows_, axis=0)
                    dd = tb(11, n)
                    r0 = c * L + g * GS
                    for p in range(NP):
                        yk_ref[r0 + 8 * p:r0 + 8 * p + 8, 128 * n:128 * n + 128] = rows_[p] * dd
                    out[n][g] = blk
                lumps.append((12 * NP + 8, run))
        return lumps

    def chain_lumps(a_):
        lumps = []
        for g in range(NCH):
            sgn = 1.0 if g < 8 else -1.0
            for n in range(NT):
                def run(tick, g=g, n=n, sgn=sgn):
                    r = g * 16
                    sl = slice(128 * n, 128 * n + 128)
                    z = 0
                    u0r = tie(u_ref[z, r:r + 8, sl], tick)
                    yr = yi = None
                    for b_ in range(a_ + 1):
                        kr = kk_ref[z + (a_ - b_), r:r + 8, sl]
                        ki = kk_ref[z + (a_ - b_), r + 8:r + 16, sl]
                        ur = u0r if b_ == 0 else u_ref[z + b_, r:r + 8, sl]
                        ui = u_ref[z + b_, r + 8:r + 16, sl]
                        tr = kr * ur - ki * ui
                        ti = kr * ui + ki * ur
                        yr = tr if yr is None else yr + tr
                        yi = ti if yi is None else yi + ti
                    if a_ == 0:
                        zr, zi = yr, yi
                    else:
                        pr = yp_ref[z + g, 0:8, sl]
                        pi = yp_ref[z + g, 8:16, sl]
                        if sgn > 0:
                            zr, zi = yr - pi, yi + pr
                        else:
                            zr, zi = yr + pi, yi - pr
                    if a_ < NCH - 1:
                        yp_ref[g, 0:8, sl] = yr
                        yp_ref[g, 8:16, sl] = yi
                    z_ref[n, a_ * 2 * L + r:a_ * 2 * L + r + 16, :] = jnp.concatenate([zr, zi], axis=0).astype(BF16)
                lumps.append((8 * (a_ + 1) + 4, run))
        return lumps

    def s1a_lumps(j, out):
        lumps = []
        for g in range(T // GS):
            for qq in range(HW):
                def run(tick, g=g, qq=qq):
                    tb = tabv()
                    r0 = j * T + g * GS
                    xs = []
                    for n in range(NT):
                        w = xw[n, pl.ds(r0 // 2 + qq, 8, stride=HW), :]
                        lo, hi = unpack2(w)
                        if n == 0:
                            lo = tie(lo, tick)
                            hi = tie(hi, tick)
                        xs.append(jnp.concatenate([lo, hi], axis=0))
                    xn = _ln_tiles(xs)
                    for n in range(NT):
                        d = tb(10, n)
                        xr_ref[r0 + 16 * qq:r0 + 16 * qq + 8, 128 * n:128 * n + 128] = xs[n][0:8] + xn[n][0:8] * d
                        xr_ref[r0 + 16 * qq + 8:r0 + 16 * qq + 16, 128 * n:128 * n + 128] = xs[n][8:16] + xn[n][8:16] * d
                    out[g * HW + qq] = jnp.concatenate(xn, axis=1).astype(BF16)
                lumps.append((95, run))
        return lumps

    def s1b_lumps(j, yconv, out):
        lumps = []
        for i in range(T // 16):
            def run(tick, i=i):
                tb = tabv()
                r0 = j * T + 16 * i
                ys, x1 = [], []
                for n in range(NT):
                    sl = slice(128 * n, 128 * n + 128)
                    yy = yconv[16 * i:16 * i + 16, sl] + yk_ref[r0:r0 + 16, sl]
                    yk_ref[r0:r0 + 16, sl] = yy
                    ys.append(yy)
                    xv = xr_ref[r0:r0 + 16, sl]
                    if n == 0:
                        xv = jnp.concatenate([tie(xv[0:8], tick), tie(xv[8:16], tick)], axis=0)
                    x1.append(xv)
                q1 = _ln_tiles(x1)
                x2 = [x1[n] + q1[n] * ys[n] for n in range(NT)]
                xn = _ln_tiles(x2)
                for n in range(NT):
                    d = tb(10, n)
                    d = jnp.concatenate([d, d], axis=0)
                    xr_ref[r0:r0 + 16, 128 * n:128 * n + 128] = x2[n] + xn[n] * d
                out[i] = jnp.concatenate(xn, axis=1).astype(BF16)
            lumps.append((200, run))
        return lumps

    def s3_lumps(j):
        lumps = []
        for g in range(T // GS):
            for qq in range(HW):
                def run(tick, g=g, qq=qq):
                    r0 = j * T + g * GS + 16 * qq
                    x3 = []
                    for n in range(NT):
                        xv = xr_ref[r0:r0 + 16, 128 * n:128 * n + 128]
                        if n == 0:
                            xv = jnp.concatenate([tie(xv[0:8], tick), tie(xv[8:16], tick)], axis=0)
                        x3.append(xv)
                    q3 = _ln_tiles(x3)
                    for n in range(NT):
                        x4 = x3[n] + q3[n] * yk_ref[r0:r0 + 16, 128 * n:128 * n + 128]
                        gb = j * T + g * GS
                        ob[n, pl.ds(gb + 2 * qq, 8, stride=NP), :] = x4[0:8]
                        ob[n, pl.ds(gb + 2 * qq + 1, 8, stride=NP), :] = x4[8:16]
                lumps.append((95, run))
        return lumps

    filler = []

    def place(ticks, dur, own, must, f0=0.0, f1=1.0, use_filler=True):
        cap = util * 4 * dur - own
        mc = sum(c for c, _ in must)
        cum = 0
        for c, fn in must:
            i = int((f0 + (f1 - f0) * cum / max(mc, 1)) * len(ticks))
            fn(ticks[min(i, len(ticks) - 1)])
            cum += c
        cap -= mc
        take = []
        while use_filler and filler and cap >= filler[0][0] * 0.5:
            c, fn = filler.pop(0)
            cap -= c
            take.append((c, fn))
        tot = sum(c for c, _ in take)
        cum = 0
        for c, fn in take:
            i = int(cum * len(ticks) / max(tot, 1))
            fn(ticks[min(i, len(ticks) - 1)])
            cum += c

    def flush(lumps):
        for c, fn in lumps:
            fn(None)

    def row_ticks(v, cols):
        out = []
        for cc in cols:
            for rr in range(0, v.shape[0], 8):
                out.append(v[rr:rr + 8, 128 * cc:128 * cc + 128])
        return out

    def job_m1(xnb, n):
        acc = None
        ticks = []
        for k in range(NT):
            t = lax.dot_general(xnb[:, 128 * k:128 * k + 128], ldbf(bbw[n, k]), _NT_DIMS,
                                preferred_element_type=F32)
            ticks += row_ticks(t, (0,))
            acc = t if acc is None else acc + t
        return acc, ticks

    def job_m2(h, k):
        w = jnp.concatenate([ldbf(crw[k]), ldbf(ciw[k])], axis=1)
        t = lax.dot_general(h, w, _NT_DIMS, preferred_element_type=F32)
        return t, row_ticks(t, range(NT))

    def job_dk(c):
        t = lax.dot_general(fn_ref[...], ldbf(skw[c]), _NT_DIMS, preferred_element_type=F32)
        kk_ref[c] = t
        return row_ticks(t, range(NT))

    def job_du(c, kvt):
        kv32 = jnp.concatenate([jnp.concatenate(kvt[n], axis=0) for n in range(NT)], axis=1)
        t = jnp.dot(fp_ref[...], kv32.astype(BF16), preferred_element_type=F32)
        u_ref[c] = t
        return row_ticks(t, range(NT))

    def job_g(j):
        ys, ticks = [], []
        for c in range(T // L):
            w0 = (j * (T // L) + c) * L
            zz = jnp.concatenate([ldbf(zw[n, w0:w0 + L, :]) for n in range(NT)], axis=1)
            y = jnp.dot(gp_ref[...], zz, preferred_element_type=F32)
            ys.append(y)
            ticks += row_ticks(y, range(NT))
        return jnp.concatenate(ys, axis=0), ticks

    def dft_jobs(cs):
        nxt = None
        for i, c in enumerate(cs):
            kvt = [[None] * (L // GS) for _ in range(NT)]
            lumps = kv_lumps(c, kvt)
            tk_ = job_dk(c)
            place(tk_, 320, 0, lumps, 0.0, 0.8)
            tu = job_du(c, kvt)
            place(tu, 320, 0, [])
            filler.extend(chain_lumps(c))

    def s5_block(xnb, carry, j, must_m1, must_m2, mid=None):
        hs, new_carry = [], []
        k1 = (len(must_m1) + NT - 1) // NT
        for n in range(NT):
            bu, ticks = job_m1(xnb, n)
            tb = tabv
            hr, hi, cy = _scan_tile(bu[:, :128], bu[:, 128:], lambda n=n: (lambda f: (lambda i: f(i, n)))(tabv()),
                                    carry[n], NP)
            new_carry.append(cy)
            hs.append(jnp.concatenate([hr, hi], axis=1).astype(BF16))
            own = 256 + (0 if n == 0 else 830)
            place(ticks, 640, own, must_m1[n * k1:(n + 1) * k1])
        extra = mid() if mid is not None else None
        m2l = must_m2(extra) if must_m2 is not None else []
        k2 = (len(m2l) + 3) // 4
        ts = []
        for k in range(NT):
            t, ticks = job_m2(hs[k], k)
            ts.append(t)
            own = 160 + (830 if (k == 0 and mid is None) else 0) + (800 if k == NT - 1 else 0)
            place(ticks, 640, own, m2l[k * k2:(k + 1) * k2] if k < 4 else [])
        acc = xr_ref[j * T:(j + 1) * T, :]
        for t in ts:
            acc = acc + t
        xr_ref[j * T:(j + 1) * T, :] = acc
        return new_carry

    zero_carry = [(jnp.zeros((8, 128), F32), jnp.zeros((8, 128), F32)) for _ in range(NT)]

    import contextlib

    def scope(name):
        return jax.named_scope(name) if opts.get("scopes") else contextlib.nullcontext()

    n1 = opts.get("n1", NB)
    n2 = opts.get("n2", NB)
    if order == "p0first":
        for q in range(NQ):
            with scope(f"dft{q}"):
                wait(("kv", q))
                dft_jobs(range(q * CQ, (q + 1) * CQ))
    with scope("bprep"):
        bprep()
    with scope("waitx"):
        wait(("x", 0))
        wait("c")
    xo = [None] * (T // 16)
    with scope("s1a0"):
        flush(s1a_lumps(0, xo))
        xnb = jnp.concatenate(xo, axis=0)
    carry = zero_carry
    for j in range(n1):
        nxt = j + 1 < NB
        if nxt and ((j + 1) * T) % RQ == 0:
            wait(("x", ((j + 1) * T) // RQ))
        xo = [None] * (T // 16)
        with scope(f"a1_{j}"):
            carry = s5_block(xnb, carry, j, [], (lambda e: s1a_lumps(j + 1, xo)) if nxt else None)
        if nxt:
            xnb = jnp.concatenate(xo, axis=0)
        if order != "p0first" and j < NQ:
            wait(("kv", j))
            dft_jobs(range(j * CQ, (j + 1) * CQ))

    carry = zero_carry
    if n2 > 0:
        need = opts.get("need0", 2)
        if opts.get("verbose"):
            print("filler before trans", len(filler), sum(c for c, _ in filler))
        with scope("trans"):
            while filler and len(filler) > (NCH - need) * NCH * NT:
                filler.pop(0)[1](None)
            yc, tg = job_g(0)
            xo = [None] * (T // 16)
            l0 = s1b_lumps(0, yc, xo)
            place(tg, 640, 320, l0)
            xnb = jnp.concatenate(xo, axis=0)
    for j in range(n2):
        nxt = j + 1 < n2
        xo = [None] * (T // 16)

        def mid():
            if not nxt:
                return None
            need = 2 * (j + 2)
            if opts.get("verbose"):
                print("filler at a2 mid", j, len(filler), sum(c for c, _ in filler))
            while filler and len(filler) > (NCH - need) * NCH * NT:
                filler.pop(0)[1](None)
            yc, tg = job_g(j + 1)
            place(tg, 640, 320 + 830, [])
            return yc

        prev3 = s3_lumps(j - 1) if j > 0 else []
        with scope(f"a2_{j}"):
            carry = s5_block(xnb, carry, j, prev3, (lambda yc: s1b_lumps(j + 1, yc, xo)) if nxt else None, mid)
        if j > 0 and not opts.get("noout") and n2 == NB:
            for n in range(NT):
                pltpu.make_async_copy(ob.at[n, pl.ds((j - 1) * T, T)],
                                      o_hbm.at[pl.ds((j - 1) * T, T), pl.ds(128 * n, 128)], osems.at[n]).start()
        if nxt:
            xnb = jnp.concatenate(xo, axis=0)
    if n2 == NB:
        with scope("tail"):
            flush(filler)
            del filler[:]
            flush(s3_lumps(NB - 1))
        for n in range(NT if not opts.get("noout") else 0):
            pltpu.make_async_copy(ob.at[n, pl.ds((NB - 1) * T, T)],
                                  o_hbm.at[pl.ds((NB - 1) * T, T), pl.ds(128 * n, 128)], osems.at[n]).start()
    else:
        for name in list(copies):
            wait(name)

        def dbody(i, c):
            for n in range(NT):
                r = pl.multiple_of(i * 128, 128)
                a_ = zw[n, pl.ds(r, 128), :]
                b_ = xr_ref[pl.ds(r, 128), 128 * n:128 * n + 128]
                c_ = yk_ref[pl.ds(r, 128), 128 * n:128 * n + 128]
                d_ = u_ref[i, 0:128, 128 * n:128 * n + 128] + kk_ref[i, 0:128, 128 * n:128 * n + 128]
                ob.at[n, pl.ds(r, 128)][...] = pltpu.bitcast(a_, F32) + b_ + c_ + d_
            return c
        lax.fori_loop(0, 16, dbody, 0)
        for n in range(NT):
            c_ = pltpu.make_async_copy(ob.at[n], o_hbm.at[:, pl.ds(128 * n, 128)], osems.at[n])
            c_.start()
    if opts.get("noout"):
        c_ = pltpu.make_async_copy(ob.at[0, 0:8], o_hbm.at[0:8, 0:128], osems.at[0])
        c_.start()
        c_.wait()
    for n in range(NT if not opts.get("noout") else 0):
        pltpu.make_async_copy(ob.at[n], o_hbm.at[:, pl.ds(128 * n, 128)], osems.at[n]).wait()
    if opts.get("verbose"):
        print("filler left", len(filler), sum(c for c, _ in filler))


def make(NP=4, **opts):
    fn_np, fp_np, gp_np = _dft_consts(NP)
    zero_np = np.concatenate([np.zeros((8, 128), np.int32), np.ones((8, 128), np.int32)])
    zs_np = np.concatenate([np.zeros(NZ - 1, np.int32), np.ones(1, np.int32)])

    @jax.jit
    def fn(A_x, A_Lambda_re, A_Lambda_im, A_B_re, A_B_im, A_C_re, A_C_im, A_log_dt, A_Dskip,
           B_q, B_k, B_v, B_shift_k, B_ssm_k, B_ssm_D):
        del B_q
        args = (A_x.reshape(S, D), A_Lambda_re, A_Lambda_im, A_B_re, A_B_im, A_C_re, A_C_im,
                A_log_dt, A_Dskip, B_k.reshape(S, D), B_v.reshape(S, D), B_shift_k.T, B_ssm_k,
                B_ssm_D, jnp.asarray(fn_np, BF16), jnp.asarray(fp_np, BF16), jnp.asarray(gp_np, BF16),
                jnp.asarray(zero_np))
        hbm = pl.BlockSpec(memory_space=pltpu.HBM)
        vm = pl.BlockSpec(memory_space=pltpu.VMEM)
        nsem = 1 + 16 + 40 + 10 + 20 + 10
        out = pl.pallas_call(
            functools.partial(_kernel, NP=NP, opts=opts),
            out_shape=jax.ShapeDtypeStruct((S, D), F32),
            in_specs=[hbm, vm, vm, hbm, hbm, hbm, hbm, vm, vm, hbm, hbm, vm, hbm, vm, vm, vm, vm, vm],
            out_specs=hbm,
            scratch_shapes=[
                pltpu.VMEM((NT, S + 16, 128), BF16),
                pltpu.VMEM((NT, S, 128), BF16),
                pltpu.VMEM((NT, S, 128), BF16),
                pltpu.VMEM((NCH, D, L), BF16),
                pltpu.VMEM((NT, D, 128), BF16),
                pltpu.VMEM((NT, D, 128), BF16),
                pltpu.VMEM((NT, D, 128), BF16),
                pltpu.VMEM((NT, D, 128), BF16),
                pltpu.VMEM((NT, NT, 256, 128), BF16),
                pltpu.VMEM((16, 8, D), F32),
                pltpu.VMEM((NCH, 2 * L, D), F32),
                pltpu.VMEM((NCH, 2 * L, D), F32),
                pltpu.VMEM((NCH, 16, D), F32),
                pltpu.VMEM((NT, NCH * 2 * L, 128), BF16),
                pltpu.VMEM((S, D), F32),
                pltpu.VMEM((S, D), F32),
                pltpu.VMEM((NT, S, 128), F32),
                pltpu.SemaphoreType.DMA((nsem,)),
                pltpu.SemaphoreType.DMA((NT,)),
            ],
            compiler_params=pltpu.CompilerParams(vmem_limit_bytes=110 * 1024 * 1024,
                                                 **({"flags": opts["flags"]} if "flags" in opts else {})),
            name="ssm_fused",
        )(*args)
        return out.reshape(1, S, D)
    return fn


pallas_interleave_layers__ssm_conv_s5__ssm_conv_h3__prompt_kernel = make()
```

```python
import functools
import numpy as np
import jax
import jax.numpy as jnp
from jax import lax
import jax.experimental.pallas as pl
import jax.experimental.pallas.tpu as pltpu

S = 2048
D = 640
L = 128
NCH = S // L
NT = D // 128
T = 256
NB = S // T
F32 = jnp.float32
BF16 = jnp.bfloat16
U32 = jnp.uint32
NZ = 1024


def _perm(np_):
    gsz = 8 * np_
    t = np.zeros(L, np.int64)
    for rho in range(L):
        g, r = divmod(rho, gsz)
        p, s = divmod(r, 8)
        t[rho] = gsz * g + np_ * s + p
    return t


def _dft_consts(np_):
    n = 2 * L
    ks = np.concatenate([np.arange(0, L, 2), np.arange(1, L, 2)])
    t = np.arange(L)
    th = 2.0 * np.pi * np.outer(ks + 0.5, t) / n
    c = np.cos(th)
    s = -np.sin(th)
    f = np.concatenate([c.reshape(L // 8, 8, L), s.reshape(L // 8, 8, L)], axis=1).reshape(2 * L, L)
    g = f.T / L
    p = _perm(np_)
    fp = f[:, p]
    gp = g[p, :]
    return (f.astype(np.float32), np.ascontiguousarray(fp).astype(np.float32),
            np.ascontiguousarray(gp).astype(np.float32))


def _ln_tiles(xs):
    s = xs[0]
    for x in xs[1:]:
        s = s + x
    m = jnp.sum(s, axis=-1, keepdims=True) * (1.0 / D)
    xc = [x - m for x in xs]
    q = xc[0] * xc[0]
    for x in xc[1:]:
        q = q + x * x
    v = jnp.sum(q, axis=-1, keepdims=True) * (1.0 / D)
    r = lax.rsqrt(v + 1e-5)
    return [x * r for x in xc]


def _cmac(br, bi, mr, mi, xr, xi):
    return br + (mr * xr - mi * xi), bi + (mr * xi + mi * xr)


def _scan_tile(bur, bui, tab, carry, np_):
    gsz = 8 * np_
    row0 = lax.broadcasted_iota(jnp.int32, (8, 128), 0) == 0
    cr, ci = carry
    outr, outi = [], []
    for g in range(T // gsz):
        lr, li = tab(8), tab(9)
        br = [bur[gsz * g + 8 * p:gsz * g + 8 * p + 8] for p in range(np_)]
        bi = [bui[gsz * g + 8 * p:gsz * g + 8 * p + 8] for p in range(np_)]
        vr, vi = br[0], bi[0]
        for p in range(1, np_):
            vr, vi = _cmac(br[p], bi[p], lr, li, vr, vi)
        for si, sh in enumerate((1, 2, 4)):
            vr, vi = _cmac(vr, vi, tab(2 * si), tab(2 * si + 1), pltpu.roll(vr, sh, 0), pltpu.roll(vi, sh, 0))
        hr, hi = _cmac(vr, vi, tab(6), tab(7), cr, ci)
        pr = jnp.where(row0, cr, pltpu.roll(hr, 1, 0))
        pi = jnp.where(row0, ci, pltpu.roll(hi, 1, 0))
        for p in range(np_ - 1):
            pr, pi = _cmac(br[p], bi[p], lr, li, pr, pi)
            outr.append(pr)
            outi.append(pi)
        outr.append(hr)
        outi.append(hi)
        cr = jnp.broadcast_to(hr[7:8], (8, 128))
        ci = jnp.broadcast_to(hi[7:8], (8, 128))
    return jnp.concatenate(outr, axis=0), jnp.concatenate(outi, axis=0), (cr, ci)


_NT_DIMS = (((1,), (1,)), ((), ()))


def _kernel(x_hbm, lre_h, lim_h, bre_hbm, bim_hbm, cre_hbm, cim_hbm, ldt_h, dsk_h,
            k_hbm, v_hbm, shk_h, ssmk_hbm, ssmd_h, fn_h, fp_h, gp_h, zero_h,
            o_hbm,
            lre_ref, lim_ref, ldt_ref, dsk_ref, ssmd_ref, shk_in, fn_ref, fp_ref, gp_ref, zero_ref,
            kb, vb, xb, sk, brb, bib, crb, cib, cc, xn_ref, tab_ref, u_ref, kk_ref, yp_ref, z_ref, yk_ref,
            xr_ref, ob, carry_ref, kvs_ref, fake_ref, sems, osems, *, NP, opts):
    GS = 8 * NP
    HW = NP // 2
    NQ = 4
    RQ = S // NQ
    CQ = NCH // NQ
    util = opts.get("util", 0.8)

    copies = {}
    idx = [0]

    def add(name, src, dst):
        c = pltpu.make_async_copy(src, dst, sems.at[idx[0]])
        idx[0] += 1
        copies.setdefault(name, []).append(c)
        c.start()

    def wait(*names):
        for name in names:
            for c in copies.pop(name):
                c.wait()

    def dma_kv(q):
        for c in range(q * CQ, (q + 1) * CQ):
            add(("kv", q), ssmk_hbm.at[:, pl.ds(L * c, L)], sk.at[c])
        for n in range(NT):
            add(("kv", q), k_hbm.at[pl.ds(RQ * q, RQ), pl.ds(128 * n, 128)], kb.at[n, pl.ds(16 + RQ * q, RQ)])
        for n in range(NT):
            add(("kv", q), v_hbm.at[pl.ds(RQ * q, RQ), pl.ds(128 * n, 128)], vb.at[n, pl.ds(RQ * q, RQ)])

    def dma_x(name, r0, r1):
        for n in range(NT):
            add(name, x_hbm.at[pl.ds(r0, r1 - r0), pl.ds(128 * n, 128)], xb.at[n, pl.ds(r0, r1 - r0)])

    import contextlib

    def scope(name):
        return jax.named_scope(name) if opts.get("scopes") else contextlib.nullcontext()

    with scope("i_p"):
        for src_, dst_ in ((lre_h, lre_ref), (lim_h, lim_ref), (ldt_h, ldt_ref), (dsk_h, dsk_ref),
                           (ssmd_h, ssmd_ref), (shk_h, shk_in), (zero_h, zero_ref)):
            add("p", src_, dst_)
    with scope("i_x0b"):
        dma_x("x0", 0, T)
        bgroups = opts.get("bgroups", ((0,), (1,), (2,), (3, 4)))
        for gi, grp in enumerate(bgroups):
            r0, nr = 128 * grp[0], 128 * len(grp)
            for k in range(NT):
                add(("b", gi), bre_hbm.at[pl.ds(r0, nr), pl.ds(128 * k, 128)], brb.at[k, pl.ds(r0, nr)])
                add(("b", gi), bim_hbm.at[pl.ds(r0, nr), pl.ds(128 * k, 128)], bib.at[k, pl.ds(r0, nr)])
            if gi == opts.get("x1after", 2):
                dma_x("x1", T, 2 * T)
    def issue_c():
        for n in range(NT):
            add("c", cre_hbm.at[:, pl.ds(128 * n, 128)], crb.at[n])
            add("c", cim_hbm.at[:, pl.ds(128 * n, 128)], cib.at[n])

    def issue_kv0():
        dma_x("x2", 2 * T, 4 * T)
        add("f", fn_h, fn_ref)
        add("f", fp_h, fp_ref)
        add("f", gp_h, gp_ref)
        dma_kv(0)

    ipos = opts.get("ipos", (0, 0))
    if ipos[0] == 0:
        issue_c()
    if ipos[1] == 0:
        issue_kv0()
    with scope("i_zero"):
        kb[:, 0:16, :] = jnp.zeros((NT, 16, 128), BF16)

    with scope("wp"):
        wait("p", "x0")
    with scope("tables"):
        lre = lre_ref[...].astype(F32).reshape(1, D)
        lim = lim_ref[...].astype(F32).reshape(1, D)
        dt = jnp.exp(ldt_ref[...].astype(F32).reshape(1, D)).astype(BF16).astype(F32)
        a = dt * lre
        b = dt * lim
        row = lax.broadcasted_iota(jnp.int32, (16, D), 0)
        nn = jnp.where(row < 8, (row + 1) * NP, 1).astype(F32)
        e = jnp.exp(a * nn)
        pr_ = e * jnp.cos(b * nn)
        pi_ = e * jnp.sin(b * nn)
        row8 = lax.broadcasted_iota(jnp.int32, (8, D), 0)
        for si, sh in enumerate((1, 2, 4)):
            tab_ref[2 * si] = jnp.where(row8 >= sh, jnp.broadcast_to(pr_[sh - 1:sh], (8, D)), 0.0)
            tab_ref[2 * si + 1] = jnp.where(row8 >= sh, jnp.broadcast_to(pi_[sh - 1:sh], (8, D)), 0.0)
        tab_ref[6] = pr_[0:8]
        tab_ref[7] = pi_[0:8]
        l1r = pr_[8:9]
        l1i = pi_[8:9]
        tab_ref[8] = jnp.broadcast_to(l1r, (8, D))
        tab_ref[9] = jnp.broadcast_to(l1i, (8, D))
        lr = l1r - 1.0
        den = lre * lre + lim * lim
        tab_ref[16] = jnp.broadcast_to(2.0 * (lr * lre + l1i * lim) / den, (8, D))
        tab_ref[17] = jnp.broadcast_to(2.0 * (l1i * lre - lr * lim) / den, (8, D))
        tab_ref[10] = jnp.broadcast_to(dsk_ref[...].astype(F32).reshape(1, D), (8, D))
        tab_ref[11] = jnp.broadcast_to(ssmd_ref[...].astype(F32).reshape(1, D), (8, D))
        shk = shk_in[...].astype(F32)
        for i in range(4):
            tab_ref[12 + i] = jnp.broadcast_to(shk[i:i + 1, :], (8, D))

    kw = kb.bitcast(U32)
    vw = vb.bitcast(U32)
    xw = xb.bitcast(U32)
    brw = brb.bitcast(U32)
    biw = bib.bitcast(U32)
    crw = crb.bitcast(U32)
    ciw = cib.bitcast(U32)
    ccw = cc.bitcast(U32)
    zw = z_ref.bitcast(U32)
    skw = sk.bitcast(U32)
    xnw = xn_ref.bitcast(U32)
    never = zero_ref[0:8, :] != 0

    def tab(i, n):
        return tab_ref[i, :, 128 * n:128 * n + 128]

    def ldbf(w):
        return pltpu.bitcast(w, BF16)

    def tie(val, tick):
        if tick is None or not opts.get("ties", True):
            return val
        return jnp.where(never, tick, val)

    def unpack2(w):
        lo = pltpu.unpack_elementwise(w, index=0, packed_dtype=BF16, unpacked_dtype=F32)
        hi = pltpu.unpack_elementwise(w, index=1, packed_dtype=BF16, unpacked_dtype=F32)
        return lo, hi

    def view(ref, start, size, align):
        if isinstance(start, int):
            return lambda idx0, lo, n: (ref[idx0][lo:lo + n] if False else None)
        return None

    class Rows:
        def __init__(self, ref, start, size, align, tiled):
            self.static = isinstance(start, int)
            self.tiled = tiled
            if self.static:
                self.ref, self.off = ref, start
            else:
                st = pl.multiple_of(start, align)
                self.ref = ref.at[:, pl.ds(st, size)] if tiled else ref.at[pl.ds(st, size)]
                self.off = 0

        def ld(self, n, r, nr, stride=None):
            o = self.off + r
            if self.tiled:
                if stride:
                    return self.ref[n, pl.ds(o, nr, stride=stride), :]
                return self.ref[n, o:o + nr, :]
            return self.ref[o:o + nr, 128 * n:128 * n + 128]

        def st(self, n, r, nr, val, stride=None):
            o = self.off + r
            if self.tiled:
                if stride:
                    self.ref[n, pl.ds(o, nr, stride=stride), :] = val
                else:
                    self.ref[n, o:o + nr, :] = val
            else:
                self.ref[o:o + nr, 128 * n:128 * n + 128] = val

    class Lead:
        def __init__(self, ref, start, size):
            if isinstance(start, int):
                self.ref, self.off = ref, start
            else:
                self.ref, self.off = ref.at[pl.ds(start, size)], 0

        def ld(self, i, r, nr, n):
            return self.ref[self.off + i, r:r + nr, 128 * n:128 * n + 128]

        def st(self, i, r, nr, n, val):
            self.ref[self.off + i, r:r + nr, 128 * n:128 * n + 128] = val

    def cprep_lumps(k):
        lumps = []
        for rb in range(D // 64):
            def run(tick, rb=rb):
                cr_, ci_ = tab(16, k), tab(17, k)
                crr = jnp.concatenate([cr_] * 2, axis=0)
                cii = jnp.concatenate([ci_] * 2, axis=0)
                for r in range(rb * 64, rb * 64 + 64, 16):
                    c_r = ldbf(crw[k, r // 2:r // 2 + 8, :]).astype(F32)
                    c_i = ldbf(ciw[k, r // 2:r // 2 + 8, :]).astype(F32)
                    if r == rb * 64:
                        c_r = jnp.concatenate([tie(c_r[0:8], tick), c_r[8:16]], axis=0)
                    cc[k, 0, r:r + 16, :] = (c_r * crr - c_i * cii).astype(BF16)
                    cc[k, 1, r:r + 16, :] = (-(c_r * cii + c_i * crr)).astype(BF16)
            lumps.append((4 * 18, run))
        return lumps

    def kv_lumps(c0, ci, kview, vview, ykv, out):
        lumps = []
        for n in range(NT):
            for g in range(L // GS):
                def run(tick, n=n, g=g):
                    w0 = ci * (L // 2) + g * GS // 2
                    cur, prev, vv = [], [], []
                    for q in range(HW):
                        cur += list(unpack2(kview.ld(n, 8 + w0 + q, 8, HW)))
                        prev += list(unpack2(kview.ld(n, 8 + w0 - HW + q, 8, HW)))
                        vv += list(unpack2(vview.ld(n, w0 + q, 8, HW)))
                    vv = [tie(x, tick) for x in vv[:1]] + vv[1:]
                    rows_ = []
                    for p in range(NP):
                        acc = None
                        for i in range(4):
                            src = cur[p - i] if p - i >= 0 else prev[NP + p - i]
                            t = src * tab(12 + i, n)
                            acc = t if acc is None else acc + t
                        rows_.append(acc * vv[p])
                    kvs_ref[out, n, g * GS:(g + 1) * GS, :] = jnp.concatenate(rows_, axis=0).astype(BF16)
                lumps.append((11 * NP + 4, run))
        return lumps

    def chain(a_, g_u, r, n, sgn, uv, kv_, get_prev, put_prev, zst, tick):
        u0r = tie(uv(0, r, n), tick)
        yr = yi = None
        for b_ in range(a_ + 1):
            kr = kv_(a_ - b_, r, n)
            ki = kv_(a_ - b_, r + 8, n)
            ur = u0r if b_ == 0 else uv(b_, r, n)
            ui = uv(b_, r + 8, n)
            tr = kr * ur - ki * ui
            ti = kr * ui + ki * ur
            yr = tr if yr is None else yr + tr
            yi = ti if yi is None else yi + ti
        if a_ == 0:
            zr, zi = yr, yi
        else:
            pr, pi = get_prev()
            if sgn > 0:
                zr, zi = yr - pi, yi + pr
            else:
                zr, zi = yr + pi, yi - pr
        if a_ < NCH - 1:
            put_prev(yr, yi)
        zst(jnp.concatenate([zr, zi], axis=0).astype(BF16))

    def chain_lumps_a(a_):
        lumps = []
        for g in range(NCH):
            sgn = 1.0 if g < 8 else -1.0
            for n in range(NT):
                def run(tick, g=g, n=n, sgn=sgn):
                    r = g * 16
                    sl = slice(128 * n, 128 * n + 128)

                    def gp_():
                        return yp_ref[g, 0:8, sl], yp_ref[g, 8:16, sl]

                    def pp_(yr, yi):
                        yp_ref[g, 0:8, sl] = yr
                        yp_ref[g, 8:16, sl] = yi

                    def zst(v):
                        z_ref[n, a_ * 2 * L + r:a_ * 2 * L + r + 16, :] = v
                    chain(a_, g, r, n, sgn, lambda i, rr, nn_: u_ref[i, rr:rr + 8, 128 * nn_:128 * nn_ + 128],
                          lambda i, rr, nn_: kk_ref[i, rr:rr + 8, 128 * nn_:128 * nn_ + 128], gp_, pp_, zst, tick)
                lumps.append((8 * (a_ + 1) + 4, run))
        return lumps

    def chain_lumps_g(g, sgn):
        if isinstance(g, int):
            uvw, kvw, zvw, r, zo = u_ref, kk_ref, z_ref, g * 16, g * 16
        else:
            gs = pl.multiple_of(g * 16, 16)
            uvw = u_ref.at[:, pl.ds(gs, 16)]
            kvw = kk_ref.at[:, pl.ds(gs, 16)]
            zvw = z_ref.at[:, pl.ds(gs, (NCH - 1) * 2 * L + 16)]
            r, zo = 0, 0
        lumps = []
        for n in range(NT):
            st = {}
            for a_ in range(NCH):
                def run(tick, n=n, a_=a_, st=st):
                    def gp_():
                        return st["pr"], st["pi"]

                    def pp_(yr, yi):
                        st["pr"], st["pi"] = yr, yi

                    def zst(v):
                        zvw[n, zo + a_ * 2 * L:zo + a_ * 2 * L + 16, :] = v
                    chain(a_, g, r, n, sgn, lambda i, rr, nn_: uvw[i, rr:rr + 8, 128 * nn_:128 * nn_ + 128],
                          lambda i, rr, nn_: kvw[i, rr:rr + 8, 128 * nn_:128 * nn_ + 128], gp_, pp_, zst, tick)
                lumps.append((8 * (a_ + 1) + 4, run))
        return lumps

    def s1a_lumps(xv, xrv, par):
        lumps = []
        for g in range(T // GS):
            for qq in range(HW):
                def run(tick, g=g, qq=qq):
                    xs = []
                    for n in range(NT):
                        lo, hi = unpack2(xv.ld(n, g * GS // 2 + qq, 8, HW))
                        if n == 0:
                            lo = tie(lo, tick)
                            hi = tie(hi, tick)
                        xs.append(jnp.concatenate([lo, hi], axis=0))
                    xn = _ln_tiles(xs)
                    r0 = g * GS + 16 * qq
                    for n in range(NT):
                        d = tab(10, n)
                        xrv.st(n, r0, 8, xs[n][0:8] + xn[n][0:8] * d)
                        xrv.st(n, r0 + 8, 8, xs[n][8:16] + xn[n][8:16] * d)
                        xn_ref[par, n, r0:r0 + 16, :] = xn[n].astype(BF16)
                lumps.append((95, run))
        return lumps

    def s1b_lumps(yconv, ykv, xrv, par):
        lumps = []
        for i in range(T // 16):
            def run(tick, i=i):
                r0 = 16 * i
                ys, x1 = [], []
                for n in range(NT):
                    yy = yconv[r0:r0 + 16, 128 * n:128 * n + 128]
                    ykv.st(n, r0, 16, yy)
                    ys.append(yy)
                    xv = xrv.ld(n, r0, 16)
                    if n == 0:
                        xv = jnp.concatenate([tie(xv[0:8], tick), tie(xv[8:16], tick)], axis=0)
                    x1.append(xv)
                q1 = _ln_tiles(x1)
                x2 = [x1[n] + q1[n] * ys[n] for n in range(NT)]
                xn = _ln_tiles(x2)
                for n in range(NT):
                    d = tab(10, n)
                    xrv.st(n, r0, 16, x2[n] + xn[n] * jnp.concatenate([d, d], axis=0))
                    xn_ref[par, n, r0:r0 + 16, :] = xn[n].astype(BF16)
            lumps.append((200, run))
        return lumps

    def s3_lumps(xrv, ykv, obv):
        lumps = []
        for g in range(T // GS):
            for qq in range(HW):
                def run(tick, g=g, qq=qq):
                    r0 = g * GS + 16 * qq
                    x3 = []
                    for n in range(NT):
                        xv = xrv.ld(n, r0, 16)
                        if n == 0:
                            xv = jnp.concatenate([tie(xv[0:8], tick), tie(xv[8:16], tick)], axis=0)
                        x3.append(xv)
                    q3 = _ln_tiles(x3)
                    for n in range(NT):
                        x4 = x3[n] + q3[n] * ykv.ld(n, r0, 16)
                        obv.st(n, g * GS + 2 * qq, 8, x4[0:8], NP)
                        obv.st(n, g * GS + 2 * qq + 1, 8, x4[8:16], NP)
                lumps.append((95, run))
        return lumps

    filler = []
    cur_util = [util]

    def spread(lumps, ticks, f0, f1):
        tot = sum(c for c, _ in lumps)
        cum = 0
        for c, fn in lumps:
            i = int((f0 + (f1 - f0) * cum / max(tot, 1)) * len(ticks))
            fn(ticks[min(i, len(ticks) - 1)])
            cum += c

    def place(ticks, dur, own, must, f0=0.0, f1=1.0):
        cap = cur_util[0] * 4 * dur - own - sum(c for c, _ in must)
        spread(must, ticks, f0, f1)
        take = []
        while filler and cap >= filler[0][0] * 0.5:
            c, fn = filler.pop(0)
            cap -= c
            take.append((c, fn))
        spread(take, ticks, 0.0, 1.0)

    def flush(lumps):
        for c, fn in lumps:
            fn(None)

    def row_ticks(v, cols):
        out = []
        for cc_ in cols:
            for rr in range(0, v.shape[0], 8):
                out.append(v[rr:rr + 8, 128 * cc_:128 * cc_ + 128])
        return out

    def job_m1(xnb, n):
        acc = None
        ticks = []
        for k in range(NT):
            w = jnp.concatenate([ldbf(brw[k, 64 * n:64 * n + 64, :]), ldbf(biw[k, 64 * n:64 * n + 64, :])], axis=0)
            t = lax.dot_general(xnb[k], w, _NT_DIMS, preferred_element_type=F32)
            ticks += row_ticks(t, (0,))
            acc = t if acc is None else acc + t
        return acc, ticks

    def job_m2(h, k):
        w = jnp.concatenate([ldbf(ccw[k, 0]), ldbf(ccw[k, 1])], axis=1)
        t = lax.dot_general(h, w, _NT_DIMS, preferred_element_type=F32)
        return t, row_ticks(t, range(NT))

    def job_dk(skv, kkv, ci):
        t = lax.dot_general(fn_ref[...], ldbf(skv.ref[skv.off + ci]), _NT_DIMS, preferred_element_type=F32)
        if kkv.off + ci == 0:
            d8 = tab_ref[11]
            dz = jnp.concatenate([d8, jnp.zeros_like(d8)], axis=0)
            t = t + jnp.concatenate([dz] * (L // 8), axis=0)
        kkv.ref[kkv.off + ci] = t
        return row_ticks(t, range(NT))

    def job_du(uv, ci, kvt):
        kvsw = kvs_ref.bitcast(U32)
        t = jnp.dot(fp_ref[...], jnp.concatenate([ldbf(kvsw[kvt, n]) for n in range(NT)], axis=1),
                    preferred_element_type=F32)
        uv.ref[uv.off + ci] = t
        return row_ticks(t, range(NT))

    def job_g(zv):
        ys, ticks = [], []
        for c in range(T // L):
            zz = jnp.concatenate([ldbf(zv.ld(n, c * L, L)) for n in range(NT)], axis=1)
            y = jnp.dot(gp_ref[...], zz, preferred_element_type=F32)
            ys.append(y)
            ticks += row_ticks(y, range(NT))
        return jnp.concatenate(ys, axis=0), ticks

    def dft_group(c0, ncs):
        kview = Rows(kw, c0 * (L // 2), ncs * (L // 2) + 8, L // 2, True)
        vview = Rows(vw, c0 * (L // 2), ncs * (L // 2), L // 2, True)
        ykv = Rows(yk_ref, c0 * L, ncs * L, L, False)
        skv, kkv, uv = Lead(skw, c0, ncs), Lead(kk_ref, c0, ncs), Lead(u_ref, c0, ncs)
        for ci in range(ncs):
            kvt = (c0 + ci) % 4
            lumps = kv_lumps(c0, ci, kview, vview, ykv, kvt)
            tk_ = job_dk(skv, kkv, ci)
            dfo = opts.get("dfo", 0)
            place(tk_, 320, dfo, lumps, 0.0, 0.8)
            tu = job_du(uv, ci, kvt)
            place(tu, 320, dfo, [])
            if isinstance(c0, int) and opts.get("mode1", "static") == "static":
                filler.extend(chain_lumps_a(c0 + ci))

    def m1_part(carry, must, par):
        xnb = [ldbf(xnw[par, k]) for k in range(NT)]
        hs, new_carry = [], []
        k1 = (len(must) + NT - 1) // NT
        for n in range(NT):
            bu, ticks = job_m1(xnb, n)
            hr, hi, cy = _scan_tile(bu[:, :128], bu[:, 128:], lambda i, n=n: tab(i, n), carry[n], NP)
            new_carry.append(cy)
            hs.append(jnp.concatenate([hr, hi], axis=1).astype(BF16))
            own = 256 + (0 if n == 0 else 830)
            place(ticks, 640, own, must[n * k1:(n + 1) * k1])
        return hs, new_carry

    def m2_part(hs, xrv, must_k, scan_tail):
        ts = []
        for k in range(NT):
            t, ticks = job_m2(hs[k], k)
            ts.append(t)
            own = 160 + (830 if (k == 0 and scan_tail) else 0) + (800 if k == NT - 1 else 0)
            place(ticks, 640, own, must_k[k])
        for n in range(NT):
            acc = xrv.ld(n, 0, T)
            for t in ts:
                acc = acc + t[:, 128 * n:128 * n + 128]
            xrv.st(n, 0, T, acc)

    def split(lumps, parts, total=NT):
        k = (len(lumps) + parts - 1) // parts
        return [lumps[i * k:(i + 1) * k] if i < parts else [] for i in range(total)]

    zero_carry = [(jnp.zeros((8, 128), F32), jnp.zeros((8, 128), F32)) for _ in range(NT)]

    def xwin(j):
        return Rows(xw, j * (T // 2), T // 2, T // 2, True)

    def rwin(ref, j):
        return Rows(ref, j * T, T, T, False)


    def barrier(fn):
        fn()

    nfake = [0]

    def issue_fakes():
        for i in range(len(opts.get("extrabar", ()))):
            add(("fake", i), zero_h, fake_ref.at[i])

    def fake_barrier():
        wait(("fake", nfake[0]))
        nfake[0] += 1

    def get_carry():
        return [(carry_ref[2 * n], carry_ref[2 * n + 1]) for n in range(NT)]

    def put_carry(c):
        for n in range(NT):
            carry_ref[2 * n] = c[n][0]
            carry_ref[2 * n + 1] = c[n][1]

    def force(n_left):
        if opts.get("verbose") and len(filler) > n_left:
            print("force", len(filler) - n_left, sum(c for c, _ in filler[:len(filler) - n_left]), "left", n_left)
        while len(filler) > n_left:
            filler.pop(0)[1](None)

    def zwin(j):
        return Rows(zw, j * (T // L) * L, (T // L) * L, L, True)

    def out_dma(j):
        for n in range(NT):
            pltpu.make_async_copy(ob.at[n, pl.ds(j * T, T)], o_hbm.at[pl.ds(j * T, T), pl.ds(128 * n, 128)],
                                  osems.at[n]).start()

    def obwin(j):
        return Rows(ob, j * T, T, T, True)

    with scope("wx0"):
        if ipos[0] == 1:
            issue_c()
    with scope("head"):
        flush(s1a_lumps(xwin(0), rwin(xr_ref, 0), 0))
    xnb0 = [ldbf(xnw[0, k]) for k in range(NT)]
    hs0, carry = [], []
    s1b1 = None
    for gi, grp in enumerate(bgroups):
        with scope(f"wb{gi}"):
            wait(("b", gi))
            if gi == opts.get("x1after", 2) + 1 or (gi == len(bgroups) - 1 and "x1" in copies):
                wait("x1")
                s1b1 = s1a_lumps(xwin(1), rwin(xr_ref, 1), 1)
        with scope(f"a1_0_{gi}"):
            for ii, n in enumerate(grp):
                bu, ticks = job_m1(xnb0, n)
                hr, hi, cy = _scan_tile(bu[:, :128], bu[:, 128:], lambda i, n=n: tab(i, n), zero_carry[n], NP)
                carry.append(cy)
                hs0.append(jnp.concatenate([hr, hi], axis=1).astype(BF16))
                must = []
                if s1b1 is not None:
                    left = NT - n
                    take = (len(s1b1) + left - 1) // left
                    must, s1b1 = s1b1[:take], s1b1[take:]
                place(ticks, 640, 256, must, 0.0, 0.7)
    xnb1 = [ldbf(xnw[1, k]) for k in range(NT)]
    hs1, carry1 = [], []
    cpos = opts.get("cpos", 4)
    for n in range(NT):
        if n == cpos:
            with scope("wc"):
                wait("c")
                issue_fakes()
                if ipos[1] == 3:
                    issue_kv0()
        with scope(f"a1_1m1_{n}"):
            bu, ticks = job_m1(xnb1, n)
            hr, hi, cy = _scan_tile(bu[:, :128], bu[:, 128:], lambda i, n=n: tab(i, n), carry[n], NP)
            carry1.append(cy)
            hs1.append(jnp.concatenate([hr, hi], axis=1).astype(BF16))
            place(ticks, 640, 256 + 830, cprep_lumps(n - cpos) if n >= cpos else [], 0.0, 0.8)
    carry = carry1
    dma_kv(1)
    dma_kv(2)
    with scope("a1_0m2"):
        nd = NT - cpos
        m2_part(hs0, rwin(xr_ref, 0), [cprep_lumps(k + nd) if k + nd < NT else [] for k in range(NT)], True)
    with scope("w_x2kv0"):
        wait(*opts.get("w0", ("x2", "f", ("kv", 0))))
    with scope("a1_1m2"):
        s1 = split(s1a_lumps(xwin(2), rwin(xr_ref, 2), 0), 4)
        m2_part(hs1, rwin(xr_ref, 1), s1, False)
        put_carry(carry)
    late_issue = [lambda: (dma_x("x3", 4 * T, S), dma_kv(3))]

    def a1_block(j):
        carry = get_carry()
        hs, carry = m1_part(carry, [], j % 2)
        put_carry(carry)
        if j + 1 < NB:
            s1 = split(s1a_lumps(xwin(j + 1), rwin(xr_ref, j + 1), (j + 1) % 2), 4)
            m2_part(hs, rwin(xr_ref, j), s1, True)
        else:
            force((NCH - 2) * NCH * NT)
            yc, tg = job_g(zwin(0))
            place(tg, 640, 160 + 830, [])
            s1 = split(s1b_lumps(yc, rwin(yk_ref, 0), rwin(xr_ref, 0), 0), 4)
            m2_part(hs, rwin(xr_ref, j), s1, False)

    dpos = opts.get("dpos", (2, 3, 4, 5))
    for j in range(2, NB):
        for q in range(NQ):
            if dpos[q] == j:
                with scope(f"dft{q}"):
                    wq = opts.get("wq", {0: (), 1: (("kv", 1), "x3"), 2: (("kv", 2), ("kv", 3)), 3: ()})
                    with scope(f"w_q{q}"):
                        wait(*wq[q])
                    if q in opts.get("extrabar", ()):
                        fake_barrier()
                    if late_issue:
                        late_issue.pop()()
                    barrier(lambda q=q: dft_group(q * CQ, CQ))
        if ("a1", j) in opts.get("extrabar", ()):
            fake_barrier()
        with scope(f"a1_{j}"):
            barrier(lambda j=j: a1_block(j))

    cur_util[0] = opts.get("util2", util)
    for n in range(NT):
        carry_ref[2 * n] = jnp.zeros((8, 128), F32)
        carry_ref[2 * n + 1] = jnp.zeros((8, 128), F32)

    def a2_block(j):
        carry = get_carry()
        prev3 = s3_lumps(rwin(xr_ref, j - 1), rwin(yk_ref, j - 1), obwin(j - 1)) if j > 0 else []
        hs, carry = m1_part(carry, prev3, j % 2)
        put_carry(carry)
        if j + 1 < NB:
            force((NCH - 2 * (j + 2)) * NCH * NT)
            yc, tg = job_g(zwin(j + 1))
            place(tg, 640, 160 + 830, [])
            s1 = split(s1b_lumps(yc, rwin(yk_ref, j + 1), rwin(xr_ref, j + 1), (j + 1) % 2), 4)
        else:
            if j > 0:
                out_dma(j - 1)
            s1 = [[]] * NT
        m2_part(hs, rwin(xr_ref, j), s1, j + 1 == NB)

    for j in range(NB):
        if ("a2", j) in opts.get("extrabar", ()):
            fake_barrier()
        with scope(f"a2_{j}"):
            barrier(lambda j=j: a2_block(j))
        if 0 < j < NB - 1:
            out_dma(j - 1)
    with scope("tail"):
        flush(filler)
        del filler[:]
        l3 = s3_lumps(rwin(xr_ref, NB - 1), rwin(yk_ref, NB - 1), obwin(NB - 1))
        ng = opts.get("tailg", 4)
        per = len(l3) // ng
        rows_per = T // ng
        for i in range(ng):
            flush(l3[i * per:(i + 1) * per])
            for n in range(NT):
                r0 = (NB - 1) * T + i * rows_per
                pltpu.make_async_copy(ob.at[n, pl.ds(r0, rows_per)],
                                      o_hbm.at[pl.ds(r0, rows_per), pl.ds(128 * n, 128)], osems.at[n]).start()
    with scope("fin"):
        for n in range(NT):
            pltpu.make_async_copy(ob.at[n, 0:S], o_hbm.at[:, pl.ds(128 * n, 128)], osems.at[n]).wait()
    if opts.get("verbose"):
        print("filler left", len(filler), sum(c for c, _ in filler))


def make(NP=4, **opts):
    fn_np, fp_np, gp_np = _dft_consts(NP)
    zero_np = np.concatenate([np.zeros((8, 128), np.int32), np.ones((8, 128), np.int32)])
    zs_np = np.concatenate([np.zeros(NZ - 1, np.int32), np.ones(1, np.int32)])

    @jax.jit
    def fn(A_x, A_Lambda_re, A_Lambda_im, A_B_re, A_B_im, A_C_re, A_C_im, A_log_dt, A_Dskip,
           B_q, B_k, B_v, B_shift_k, B_ssm_k, B_ssm_D):
        del B_q
        args = (A_x.reshape(S, D), A_Lambda_re, A_Lambda_im, A_B_re, A_B_im, A_C_re, A_C_im,
                A_log_dt, A_Dskip, B_k.reshape(S, D), B_v.reshape(S, D), B_shift_k.T, B_ssm_k,
                B_ssm_D, jnp.asarray(fn_np, BF16), jnp.asarray(fp_np, BF16), jnp.asarray(gp_np, BF16),
                jnp.asarray(zero_np))
        hbm = pl.BlockSpec(memory_space=pltpu.HBM)
        vm = pl.BlockSpec(memory_space=pltpu.VMEM)
        nsem = 7 + 10 + 50 + 10 + 3 + 56 + 10 + 16
        out = pl.pallas_call(
            functools.partial(_kernel, NP=NP, opts=opts),
            out_shape=jax.ShapeDtypeStruct((S, D), F32),
            in_specs=[hbm] * 18,
            out_specs=hbm,
            scratch_shapes=[
                pltpu.VMEM((D,), BF16), pltpu.VMEM((D,), BF16), pltpu.VMEM((D,), BF16),
                pltpu.VMEM((D,), BF16), pltpu.VMEM((D,), BF16),
                pltpu.VMEM((4, D), BF16),
                pltpu.VMEM((2 * L, L), BF16), pltpu.VMEM((2 * L, L), BF16), pltpu.VMEM((L, 2 * L), BF16),
                pltpu.VMEM((16, 128), jnp.int32),
                pltpu.VMEM((NT, S + 16, 128), BF16),
                pltpu.VMEM((NT, S, 128), BF16),
                pltpu.VMEM((NT, S, 128), BF16),
                pltpu.VMEM((NCH, D, L), BF16),
                pltpu.VMEM((NT, D, 128), BF16),
                pltpu.VMEM((NT, D, 128), BF16),
                pltpu.VMEM((NT, D, 128), BF16),
                pltpu.VMEM((NT, D, 128), BF16),
                pltpu.VMEM((NT, 2, D, 128), BF16),
                pltpu.VMEM((2, NT, T, 128), BF16),
                pltpu.VMEM((18, 8, D), F32),
                pltpu.VMEM((NCH, 2 * L, D), F32),
                pltpu.VMEM((NCH, 2 * L, D), F32),
                pltpu.VMEM((NCH, 16, D), F32),
                pltpu.VMEM((NT, NCH * 2 * L, 128), BF16),
                pltpu.VMEM((S, D), F32),
                pltpu.VMEM((S + T, D), F32),
                pltpu.VMEM((NT, S, 128), F32),
                pltpu.VMEM((2 * NT, 8, 128), F32),
                pltpu.VMEM((4, NT, L, 128), BF16),
                pltpu.VMEM((16, 16, 128), jnp.int32),
                pltpu.SemaphoreType.DMA((nsem,)),
                pltpu.SemaphoreType.DMA((NT,)),
            ],
            compiler_params=pltpu.CompilerParams(vmem_limit_bytes=110 * 1024 * 1024,
                                                 **({"flags": opts["flags"]} if "flags" in opts else {})),
            name="ssm_fused",
        )(*args)
        return out.reshape(1, S, D)
    return fn


pallas_interleave_layers__ssm_conv_s5__ssm_conv_h3__prompt_kernel = make(
    ipos=(1, 3), util=0.72, util2=0.55, extrabar=(('a1', 2), ('a1', 3), ('a1', 4), ('a1', 5)), w0=('x2',),
    wq={0: ('f', ('kv', 0)), 1: (('kv', 1), 'x3'), 2: (('kv', 2),), 3: (('kv', 3),)})
```

```python
import functools
import numpy as np
import jax
import jax.numpy as jnp
from jax import lax
import jax.experimental.pallas as pl
import jax.experimental.pallas.tpu as pltpu

S = 2048
D = 640
L = 128
NCH = S // L
NT = D // 128
T = 256
NB = S // T
F32 = jnp.float32
BF16 = jnp.bfloat16
U32 = jnp.uint32
NSEM = 24


def _perm(np_):
    gsz = 8 * np_
    t = np.zeros(L, np.int64)
    for rho in range(L):
        g, r = divmod(rho, gsz)
        p, s = divmod(r, 8)
        t[rho] = gsz * g + np_ * s + p
    return t


def _dft_consts(np_):
    n = 2 * L
    ks = np.concatenate([np.arange(0, L, 2), np.arange(1, L, 2)])
    t = np.arange(L)
    th = 2.0 * np.pi * np.outer(ks + 0.5, t) / n
    c = np.cos(th)
    s = -np.sin(th)
    f = np.concatenate([c.reshape(L // 8, 8, L), s.reshape(L // 8, 8, L)], axis=1).reshape(2 * L, L)
    g = f.T / L
    p = _perm(np_)
    fp = f[:, p]
    gp = g[p, :]
    return (f.astype(np.float32), np.ascontiguousarray(fp).astype(np.float32),
            np.ascontiguousarray(gp).astype(np.float32))


def _ln_tiles(xs):
    s = xs[0]
    for x in xs[1:]:
        s = s + x
    m = jnp.sum(s, axis=-1, keepdims=True) * (1.0 / D)
    xc = [x - m for x in xs]
    q = xc[0] * xc[0]
    for x in xc[1:]:
        q = q + x * x
    v = jnp.sum(q, axis=-1, keepdims=True) * (1.0 / D)
    r = lax.rsqrt(v + 1e-5)
    return [x * r for x in xc]


def _cmac(br, bi, mr, mi, xr, xi):
    return br + (mr * xr - mi * xi), bi + (mr * xi + mi * xr)


def _scan_tile(bur, bui, tab, carry, np_):
    gsz = 8 * np_
    row0 = lax.broadcasted_iota(jnp.int32, (8, 128), 0) == 0
    cr, ci = carry
    outr, outi = [], []
    for g in range(T // gsz):
        lr, li = tab(8), tab(9)
        br = [bur[gsz * g + 8 * p:gsz * g + 8 * p + 8] for p in range(np_)]
        bi = [bui[gsz * g + 8 * p:gsz * g + 8 * p + 8] for p in range(np_)]
        vr, vi = br[0], bi[0]
        for p in range(1, np_):
            vr, vi = _cmac(br[p], bi[p], lr, li, vr, vi)
        for si, sh in enumerate((1, 2, 4)):
            vr, vi = _cmac(vr, vi, tab(2 * si), tab(2 * si + 1), pltpu.roll(vr, sh, 0), pltpu.roll(vi, sh, 0))
        hr, hi = _cmac(vr, vi, tab(6), tab(7), cr, ci)
        pr = jnp.where(row0, cr, pltpu.roll(hr, 1, 0))
        pi = jnp.where(row0, ci, pltpu.roll(hi, 1, 0))
        for p in range(np_ - 1):
            pr, pi = _cmac(br[p], bi[p], lr, li, pr, pi)
            outr.append(pr)
            outi.append(pi)
        outr.append(hr)
        outi.append(hi)
        cr = jnp.broadcast_to(hr[7:8], (8, 128))
        ci = jnp.broadcast_to(hi[7:8], (8, 128))
    return jnp.concatenate(outr, axis=0), jnp.concatenate(outi, axis=0), (cr, ci)


_NT_DIMS = (((1,), (1,)), ((), ()))


def _kernel(x_hbm, lre_h, lim_h, bre_hbm, bim_hbm, cre_hbm, cim_hbm, ldt_h, dsk_h,
            k_hbm, v_hbm, shk_h, ssmk_hbm, ssmd_h, fn_h, fp_h, gp_h, zero_h,
            o_hbm,
            lre_ref, lim_ref, ldt_ref, dsk_ref, ssmd_ref, shk_in, fn_ref, fp_ref, gp_ref, zero_ref,
            kb, vb, xb, sk, brb, bib, crb, cib, cc, xn_ref, tab_ref, u_ref, kk_ref, yp_ref, z_ref, yk_ref,
            xr_ref, ob, carry_ref, kvs_ref, fake_ref, sems, osems, *, NP, opts):
    GS = 8 * NP
    HW = NP // 2
    NQ = 4
    RQ = S // NQ
    CQ = NCH // NQ
    util = opts.get("util", 0.72)

    copies = {}
    idx = [0]

    semid = {}

    def add(name, src, dst):
        if name not in semid:
            semid[name] = len(semid)
            assert semid[name] < NSEM
        c = pltpu.make_async_copy(src, dst, sems.at[semid[name]])
        copies.setdefault(name, []).append(c)
        c.start()

    def wait(*names):
        for name in names:
            for c in copies.pop(name):
                c.wait()

    def dma_kv(q):
        for c in range(q * CQ, (q + 1) * CQ):
            add(("kv", q), ssmk_hbm.at[:, pl.ds(L * c, L)], sk.at[c])
        for n in range(NT):
            add(("kv", q), k_hbm.at[pl.ds(RQ * q, RQ), pl.ds(128 * n, 128)], kb.at[n, pl.ds(16 + RQ * q, RQ)])
        for n in range(NT):
            add(("kv", q), v_hbm.at[pl.ds(RQ * q, RQ), pl.ds(128 * n, 128)], vb.at[n, pl.ds(RQ * q, RQ)])

    def dma_x(name, r0, r1):
        for n in range(NT):
            add(name, x_hbm.at[pl.ds(r0, r1 - r0), pl.ds(128 * n, 128)], xb.at[n, pl.ds(r0, r1 - r0)])

    import contextlib

    def scope(name):
        sc = opts.get("scopes")
        if sc == "seg":
            ok = name in ("wp", "wb0", "wb1", "wb2", "wb3", "wc", "w_x2kv0", "dft0", "dft1", "dft2", "dft3",
                          "a1_2", "a1_3", "a1_4", "a1_0m2", "a1_1m2", "a1_0_0", "a1_0_1", "a1_0_2", "big", "fin", "a1_6", "a2_0", "a2_2", "a2_4", "a2_6", "tail")
            return jax.named_scope(name) if ok else contextlib.nullcontext()
        return jax.named_scope(name) if sc else contextlib.nullcontext()

    with scope("i_p"):
        for src_, dst_ in ((lre_h, lre_ref), (lim_h, lim_ref), (ldt_h, ldt_ref), (dsk_h, dsk_ref),
                           (ssmd_h, ssmd_ref), (shk_h, shk_in), (zero_h, zero_ref)):
            add("p", src_, dst_)
    with scope("i_x0b"):
        dma_x("x0", 0, 2 * T)
        bgroups = opts.get("bgroups", ((0,), (1, 2), (3, 4)))
        for gi, grp in enumerate(bgroups):
            r0, nr = 128 * grp[0], 128 * len(grp)
            for k in range(NT):
                add(("b", gi), bre_hbm.at[pl.ds(r0, nr), pl.ds(128 * k, 128)], brb.at[k, pl.ds(r0, nr)])
                add(("b", gi), bim_hbm.at[pl.ds(r0, nr), pl.ds(128 * k, 128)], bib.at[k, pl.ds(r0, nr)])
    csplit = opts.get("csplit", 5)

    def issue_c():
        for n in range(NT):
            nm = ("c", 0) if n < csplit else ("c", 1)
            add(nm, cre_hbm.at[:, pl.ds(128 * n, 128)], crb.at[n])
            add(nm, cim_hbm.at[:, pl.ds(128 * n, 128)], cib.at[n])

    def issue_kv0():
        dma_x(("kv", 0), 2 * T, 4 * T)
        add(("kv", 0), fn_h, fn_ref)
        add(("kv", 0), fp_h, fp_ref)
        add(("kv", 0), gp_h, gp_ref)
        dma_kv(0)

    ipos = opts.get("ipos", (1, 3))
    if ipos[0] == 0:
        issue_c()
    if ipos[1] == 0:
        issue_kv0()
    with scope("i_zero"):
        kb[:, 0:16, :] = jnp.zeros((NT, 16, 128), BF16)

    with scope("wp"):
        wait("p")
    with scope("tables"):
        lre = lre_ref[...].astype(F32).reshape(1, D)
        lim = lim_ref[...].astype(F32).reshape(1, D)
        dt = jnp.exp(ldt_ref[...].astype(F32).reshape(1, D)).astype(BF16).astype(F32)
        a = dt * lre
        b = dt * lim
        row = lax.broadcasted_iota(jnp.int32, (16, D), 0)
        nn = jnp.where(row < 8, (row + 1) * NP, 1).astype(F32)
        e = jnp.exp(a * nn)
        pr_ = e * jnp.cos(b * nn)
        pi_ = e * jnp.sin(b * nn)
        row8 = lax.broadcasted_iota(jnp.int32, (8, D), 0)
        for si, sh in enumerate((1, 2, 4)):
            tab_ref[2 * si] = jnp.where(row8 >= sh, jnp.broadcast_to(pr_[sh - 1:sh], (8, D)), 0.0)
            tab_ref[2 * si + 1] = jnp.where(row8 >= sh, jnp.broadcast_to(pi_[sh - 1:sh], (8, D)), 0.0)
        tab_ref[6] = pr_[0:8]
        tab_ref[7] = pi_[0:8]
        l1r = pr_[8:9]
        l1i = pi_[8:9]
        tab_ref[8] = jnp.broadcast_to(l1r, (8, D))
        tab_ref[9] = jnp.broadcast_to(l1i, (8, D))
        lr = l1r - 1.0
        den = lre * lre + lim * lim
        tab_ref[16] = jnp.broadcast_to(2.0 * (lr * lre + l1i * lim) / den, (8, D))
        tab_ref[17] = jnp.broadcast_to(2.0 * (l1i * lre - lr * lim) / den, (8, D))
        tab_ref[10] = jnp.broadcast_to(dsk_ref[...].astype(F32).reshape(1, D), (8, D))
        tab_ref[11] = jnp.broadcast_to(ssmd_ref[...].astype(F32).reshape(1, D), (8, D))
        shk = shk_in[...].astype(F32)
        for i in range(4):
            tab_ref[12 + i] = jnp.broadcast_to(shk[i:i + 1, :], (8, D))

    kw = kb.bitcast(U32)
    vw = vb.bitcast(U32)
    xw = xb.bitcast(U32)
    brw = brb.bitcast(U32)
    biw = bib.bitcast(U32)
    crw = crb.bitcast(U32)
    ciw = cib.bitcast(U32)
    ccw = cc.bitcast(U32)
    zw = z_ref.bitcast(U32)
    skw = sk.bitcast(U32)
    xnw = xn_ref.bitcast(U32)
    never = zero_ref[0:8, :] != 0

    def tab(i, n):
        return tab_ref[i, :, 128 * n:128 * n + 128]

    def ldbf(w):
        return pltpu.bitcast(w, BF16)

    def tie(val, tick):
        if tick is None or not opts.get("ties", True):
            return val
        return jnp.where(never, tick, val)

    def unpack2(w):
        lo = pltpu.unpack_elementwise(w, index=0, packed_dtype=BF16, unpacked_dtype=F32)
        hi = pltpu.unpack_elementwise(w, index=1, packed_dtype=BF16, unpacked_dtype=F32)
        return lo, hi

    class Rows:
        def __init__(self, ref, start, size, align, tiled):
            self.static = isinstance(start, int)
            self.tiled = tiled
            if self.static:
                self.ref, self.off = ref, start
            else:
                st = pl.multiple_of(start, align)
                self.ref = ref.at[:, pl.ds(st, size)] if tiled else ref.at[pl.ds(st, size)]
                self.off = 0

        def ld(self, n, r, nr, stride=None):
            o = self.off + r
            if self.tiled:
                if stride:
                    return self.ref[n, pl.ds(o, nr, stride=stride), :]
                return self.ref[n, o:o + nr, :]
            return self.ref[o:o + nr, 128 * n:128 * n + 128]

        def st(self, n, r, nr, val, stride=None):
            o = self.off + r
            if self.tiled:
                if stride:
                    self.ref[n, pl.ds(o, nr, stride=stride), :] = val
                else:
                    self.ref[n, o:o + nr, :] = val
            else:
                self.ref[o:o + nr, 128 * n:128 * n + 128] = val

    class Lead:
        def __init__(self, ref, start, size):
            if isinstance(start, int):
                self.ref, self.off = ref, start
            else:
                self.ref, self.off = ref.at[pl.ds(start, size)], 0

        def ld(self, i, r, nr, n):
            return self.ref[self.off + i, r:r + nr, 128 * n:128 * n + 128]

        def st(self, i, r, nr, n, val):
            self.ref[self.off + i, r:r + nr, 128 * n:128 * n + 128] = val

    def cprep_lumps(k):
        lumps = []
        for rb in range(D // 64):
            def run(tick, rb=rb):
                cr_, ci_ = tab(16, k), tab(17, k)
                crr = jnp.concatenate([cr_] * 2, axis=0)
                cii = jnp.concatenate([ci_] * 2, axis=0)
                for r in range(rb * 64, rb * 64 + 64, 16):
                    c_r = ldbf(crw[k, r // 2:r // 2 + 8, :]).astype(F32)
                    c_i = ldbf(ciw[k, r // 2:r // 2 + 8, :]).astype(F32)
                    if r == rb * 64:
                        c_r = jnp.concatenate([tie(c_r[0:8], tick), c_r[8:16]], axis=0)
                    cc[k, 0, r:r + 16, :] = (c_r * crr - c_i * cii).astype(BF16)
                    cc[k, 1, r:r + 16, :] = (-(c_r * cii + c_i * crr)).astype(BF16)
            lumps.append((4 * 18, run))
        return lumps

    def kv_lumps(c0, ci, kview, vview, ykv, out):
        lumps = []
        for n in range(NT):
            for g in range(L // GS):
                def run(tick, n=n, g=g):
                    w0 = ci * (L // 2) + g * GS // 2
                    cur, prev, vv = [], [], []
                    for q in range(HW):
                        cur += list(unpack2(kview.ld(n, 8 + w0 + q, 8, HW)))
                        prev += list(unpack2(kview.ld(n, 8 + w0 - HW + q, 8, HW)))
                        vv += list(unpack2(vview.ld(n, w0 + q, 8, HW)))
                    vv = [tie(x, tick) for x in vv[:1]] + vv[1:]
                    rows_ = []
                    for p in range(NP):
                        acc = None
                        for i in range(4):
                            src = cur[p - i] if p - i >= 0 else prev[NP + p - i]
                            t = src * tab(12 + i, n)
                            acc = t if acc is None else acc + t
                        rows_.append(acc * vv[p])
                    kvs_ref[out, n, g * GS:(g + 1) * GS, :] = jnp.concatenate(rows_, axis=0).astype(BF16)
                lumps.append((11 * NP + 4, run))
        return lumps

    def chain(a_, g_u, r, n, sgn, uv, kv_, get_prev, put_prev, zst, tick):
        u0r = tie(uv(0, r, n), tick)
        yr = yi = None
        for b_ in range(a_ + 1):
            kr = kv_(a_ - b_, r, n)
            ki = kv_(a_ - b_, r + 8, n)
            ur = u0r if b_ == 0 else uv(b_, r, n)
            ui = uv(b_, r + 8, n)
            tr = kr * ur - ki * ui
            ti = kr * ui + ki * ur
            yr = tr if yr is None else yr + tr
            yi = ti if yi is None else yi + ti
        if a_ == 0:
            zr, zi = yr, yi
        else:
            pr, pi = get_prev()
            if sgn > 0:
                zr, zi = yr - pi, yi + pr
            else:
                zr, zi = yr + pi, yi - pr
        if a_ < NCH - 1:
            put_prev(yr, yi)
        zst(jnp.concatenate([zr, zi], axis=0).astype(BF16))

    def chain_lumps_a(a_):
        lumps = []
        for g in range(NCH):
            sgn = 1.0 if g < 8 else -1.0
            for n in range(NT):
                def run(tick, g=g, n=n, sgn=sgn):
                    r = g * 16
                    sl = slice(128 * n, 128 * n + 128)

                    def gp_():
                        return yp_ref[g, 0:8, sl], yp_ref[g, 8:16, sl]

                    def pp_(yr, yi):
                        yp_ref[g, 0:8, sl] = yr
                        yp_ref[g, 8:16, sl] = yi

                    def zst(v):
                        z_ref[n, a_ * 2 * L + r:a_ * 2 * L + r + 16, :] = v
                    chain(a_, g, r, n, sgn, lambda i, rr, nn_: u_ref[i, rr:rr + 8, 128 * nn_:128 * nn_ + 128],
                          lambda i, rr, nn_: kk_ref[i, rr:rr + 8, 128 * nn_:128 * nn_ + 128], gp_, pp_, zst, tick)
                lumps.append((8 * (a_ + 1) + 4, run))
        return lumps

    def chain_lumps_g(g, sgn):
        if isinstance(g, int):
            uvw, kvw, zvw, r, zo = u_ref, kk_ref, z_ref, g * 16, g * 16
        else:
            gs = pl.multiple_of(g * 16, 16)
            uvw = u_ref.at[:, pl.ds(gs, 16)]
            kvw = kk_ref.at[:, pl.ds(gs, 16)]
            zvw = z_ref.at[:, pl.ds(gs, (NCH - 1) * 2 * L + 16)]
            r, zo = 0, 0
        lumps = []
        for n in range(NT):
            st = {}
            for a_ in range(NCH):
                def run(tick, n=n, a_=a_, st=st):
                    def gp_():
                        return st["pr"], st["pi"]

                    def pp_(yr, yi):
                        st["pr"], st["pi"] = yr, yi

                    def zst(v):
                        zvw[n, zo + a_ * 2 * L:zo + a_ * 2 * L + 16, :] = v
                    chain(a_, g, r, n, sgn, lambda i, rr, nn_: uvw[i, rr:rr + 8, 128 * nn_:128 * nn_ + 128],
                          lambda i, rr, nn_: kvw[i, rr:rr + 8, 128 * nn_:128 * nn_ + 128], gp_, pp_, zst, tick)
                lumps.append((8 * (a_ + 1) + 4, run))
        return lumps

    def s1a_lumps(xv, xrv, par):
        lumps = []
        for g in range(T // GS):
            for qq in range(HW):
                def run(tick, g=g, qq=qq):
                    xs = []
                    for n in range(NT):
                        lo, hi = unpack2(xv.ld(n, g * GS // 2 + qq, 8, HW))
                        if n == 0:
                            lo = tie(lo, tick)
                            hi = tie(hi, tick)
                        xs.append(jnp.concatenate([lo, hi], axis=0))
                    xn = _ln_tiles(xs)
                    r0 = g * GS + 16 * qq
                    for n in range(NT):
                        d = tab(10, n)
                        xrv.st(n, r0, 8, xs[n][0:8] + xn[n][0:8] * d)
                        xrv.st(n, r0 + 8, 8, xs[n][8:16] + xn[n][8:16] * d)
                        xn_ref[par, n, r0:r0 + 16, :] = xn[n].astype(BF16)
                lumps.append((95, run))
        return lumps

    def s1b_lumps(yconv, ykv, xrv, par):
        lumps = []
        for i in range(T // 16):
            def run(tick, i=i):
                r0 = 16 * i
                ys, x1 = [], []
                for n in range(NT):
                    yy = yconv[r0:r0 + 16, 128 * n:128 * n + 128]
                    ykv.st(n, r0, 16, yy)
                    ys.append(yy)
                    xv = xrv.ld(n, r0, 16)
                    if n == 0:
                        xv = jnp.concatenate([tie(xv[0:8], tick), tie(xv[8:16], tick)], axis=0)
                    x1.append(xv)
                q1 = _ln_tiles(x1)
                x2 = [x1[n] + q1[n] * ys[n] for n in range(NT)]
                xn = _ln_tiles(x2)
                for n in range(NT):
                    d = tab(10, n)
                    xrv.st(n, r0, 16, x2[n] + xn[n] * jnp.concatenate([d, d], axis=0))
                    xn_ref[par, n, r0:r0 + 16, :] = xn[n].astype(BF16)
            lumps.append((200, run))
        return lumps

    def s3_lumps(xrv, ykv, obv):
        lumps = []
        for g in range(T // GS):
            for qq in range(HW):
                def run(tick, g=g, qq=qq):
                    r0 = g * GS + 16 * qq
                    x3 = []
                    for n in range(NT):
                        xv = xrv.ld(n, r0, 16)
                        if n == 0:
                            xv = jnp.concatenate([tie(xv[0:8], tick), tie(xv[8:16], tick)], axis=0)
                        x3.append(xv)
                    q3 = _ln_tiles(x3)
                    for n in range(NT):
                        x4 = x3[n] + q3[n] * ykv.ld(n, r0, 16)
                        obv.st(n, g * GS + 2 * qq, 8, x4[0:8], NP)
                        obv.st(n, g * GS + 2 * qq + 1, 8, x4[8:16], NP)
                lumps.append((95, run))
        return lumps

    filler = []
    cur_util = [util]
    jobno = [0]
    jobdur = []

    def spread(lumps, ticks, f0, f1):
        tot = sum(c for c, _ in lumps)
        cum = 0
        for c, fn in lumps:
            i = int((f0 + (f1 - f0) * cum / max(tot, 1)) * len(ticks))
            fn(ticks[min(i, len(ticks) - 1)])
            cum += c

    def place(ticks, dur, own, must, f0=0.0, f1=1.0):
        cal = opts.get("own")
        if cal is not None:
            cap = cur_util[0] * 4 * dur - cal[jobno[0]]
        else:
            cap = cur_util[0] * 4 * dur - own - sum(c for c, _ in must)
        jobno[0] += 1
        spread(must, ticks, f0, f1)
        take = []
        while filler and cap >= filler[0][0] * 0.5:
            c, fn = filler.pop(0)
            cap -= c
            take.append((c, fn))
        spread(take, ticks, 0.0, 1.0)
        jobdur.append(dur)

    def flush(lumps):
        for c, fn in lumps:
            fn(None)

    def row_ticks(v, cols):
        out = []
        for cc_ in cols:
            for rr in range(0, v.shape[0], 8):
                out.append(v[rr:rr + 8, 128 * cc_:128 * cc_ + 128])
        return out

    oz_ = pl.program_id(0) if opts.get("opq_st", False) else 0
    def job_m1(xnb, n):
        acc = None
        ticks = []
        for k in range(NT):
            w = jnp.concatenate([ldbf(brw[k, 64 * n:64 * n + 64, :]), ldbf(biw[k, 64 * n:64 * n + 64, :])], axis=0)
            t = lax.dot_general(xnb[k], w, _NT_DIMS, preferred_element_type=F32)
            ticks += row_ticks(t, (0,))
            acc = t if acc is None else acc + t
        return acc, ticks

    def job_m2(h, k):
        w = jnp.concatenate([ldbf(ccw[k, 0]), ldbf(ccw[k, 1])], axis=1)
        t = lax.dot_general(h, w, _NT_DIMS, preferred_element_type=F32)
        return t, row_ticks(t, range(NT))

    def job_dk(skv, kkv, ci):
        t = lax.dot_general(fn_ref[...], ldbf(skv.ref[skv.off + ci]), _NT_DIMS, preferred_element_type=F32)
        if kkv.off + ci == 0:
            d8 = tab_ref[11]
            dz = jnp.concatenate([d8, jnp.zeros_like(d8)], axis=0)
            t = t + jnp.concatenate([dz] * (L // 8), axis=0)
        kkv.ref[oz_ + kkv.off + ci] = t
        return row_ticks(t, range(NT))

    def job_du(uv, ci, kvt):
        kvsw = kvs_ref.bitcast(U32)
        t = jnp.dot(fp_ref[...], jnp.concatenate([ldbf(kvsw[kvt, n]) for n in range(NT)], axis=1),
                    preferred_element_type=F32)
        uv.ref[oz_ + uv.off + ci] = t
        return row_ticks(t, range(NT))

    def job_g(zv):
        ys, ticks = [], []
        for c in range(T // L):
            zz = jnp.concatenate([ldbf(zv.ld(n, c * L, L)) for n in range(NT)], axis=1)
            y = jnp.dot(gp_ref[...], zz, preferred_element_type=F32)
            ys.append(y)
            ticks += row_ticks(y, range(NT))
        return jnp.concatenate(ys, axis=0), ticks

    def dft_group(c0, ncs, extra=()):
        kview = Rows(kw, c0 * (L // 2), ncs * (L // 2) + 8, L // 2, True)
        vview = Rows(vw, c0 * (L // 2), ncs * (L // 2), L // 2, True)
        ykv = Rows(yk_ref, c0 * L, ncs * L, L, False)
        skv, kkv, uv = Lead(skw, c0, ncs), Lead(kk_ref, c0, ncs), Lead(u_ref, c0, ncs)
        for ci in range(ncs):
            kvt = (c0 + ci) % 4
            lumps = kv_lumps(c0, ci, kview, vview, ykv, kvt)
            tk_ = job_dk(skv, kkv, ci)
            dfo = opts.get("dfo", 0)
            place(tk_, 320, dfo, lumps, 0.0, 0.8)
            tu = job_du(uv, ci, kvt)
            ne = (len(extra) + ncs - 1) // ncs
            place(tu, 320, dfo, list(extra[ci * ne:(ci + 1) * ne]))
            if not opts.get("nofill"):
                filler.extend(chain_lumps_a(c0 + ci))

    def m1_part(carry, must, par):
        xnb = [ldbf(xnw[par, k]) for k in range(NT)]
        hs, new_carry = [], []
        k1 = (len(must) + NT - 1) // NT
        for n in range(NT):
            bu, ticks = job_m1(xnb, n)
            hr, hi, cy = _scan_tile(bu[:, :128], bu[:, 128:], lambda i, n=n: tab(i, n), carry[n], NP)
            new_carry.append(cy)
            hs.append(jnp.concatenate([hr, hi], axis=1).astype(BF16))
            own = 256 + (0 if n == 0 else 830)
            place(ticks, 640, own, must[n * k1:(n + 1) * k1])
        return hs, new_carry

    def m2_part(hs, xrv, must_k, scan_tail, pre={}):
        ts = []
        for k in range(NT):
            if k in pre:
                pre[k]()
            t, ticks = job_m2(hs[k], k)
            ts.append(t)
            own = 160 + (830 if (k == 0 and scan_tail) else 0) + (800 if k == NT - 1 else 0)
            place(ticks, 640, own, must_k[k])
        for n in range(NT):
            acc = xrv.ld(n, 0, T)
            for t in ts:
                acc = acc + t[:, 128 * n:128 * n + 128]
            xrv.st(n, 0, T, acc)

    def split(lumps, parts, total=NT):
        k = (len(lumps) + parts - 1) // parts
        return [lumps[i * k:(i + 1) * k] if i < parts else [] for i in range(total)]

    zero_carry = [(jnp.zeros((8, 128), F32), jnp.zeros((8, 128), F32)) for _ in range(NT)]

    def xwin(j):
        return Rows(xw, j * (T // 2), T // 2, T // 2, True)

    def rwin(ref, j):
        return Rows(ref, j * T, T, T, False)


    def barrier(fn):
        fn()

    nfake = [0]

    def issue_fakes():
        for i in range(len(opts.get("extrabar", (("a1", 2), ("a1", 3), ("a1", 4), ("a1", 5))))):
            add(("fake", i), zero_h, fake_ref.at[i])

    def fake_barrier():
        wait(("fake", nfake[0]))
        nfake[0] += 1

    def get_carry():
        return [(carry_ref[2 * n], carry_ref[2 * n + 1]) for n in range(NT)]

    def put_carry(c):
        for n in range(NT):
            carry_ref[2 * n] = c[n][0]
            carry_ref[2 * n + 1] = c[n][1]

    def force(n_left):
        if opts.get("verbose") and len(filler) > n_left:
            print("force", len(filler) - n_left, sum(c for c, _ in filler[:len(filler) - n_left]), "left", n_left)
        while len(filler) > n_left:
            filler.pop(0)[1](None)

    def zwin(j):
        return Rows(zw, j * (T // L) * L, (T // L) * L, L, True)

    def out_dma(j):
        for n in range(NT):
            pltpu.make_async_copy(ob.at[n, pl.ds(j * T, T)], o_hbm.at[pl.ds(j * T, T), pl.ds(128 * n, 128)],
                                  osems.at[0]).start()

    def obwin(j):
        return Rows(ob, j * T, T, T, True)

    with scope("wx0"):
        wait("x0")
        if ipos[0] == 1:
            issue_c()
    with scope("head"):
        flush(s1a_lumps(xwin(0), rwin(xr_ref, 0), 0))
    xnb0 = [ldbf(xnw[0, k]) for k in range(NT)]
    xnb1 = None
    hs0, hs1, carry = [], [], []
    s1b1 = s1a_lumps(xwin(1), rwin(xr_ref, 1), 1)
    cpos = opts.get("cpos", 5)
    for gi, grp in enumerate(bgroups):
        with scope(f"wb{gi}"):
            wait(("b", gi))
        with scope(f"a1_0_{gi}"):
            for n in grp:
                bu, ticks = job_m1(xnb0, n)
                hr, hi, cy = _scan_tile(bu[:, :128], bu[:, 128:], lambda i, n=n: tab(i, n), zero_carry[n], NP)
                hs0.append(jnp.concatenate([hr, hi], axis=1).astype(BF16))
                place(ticks, 640, 256, s1b1 if n == 0 else [], 0.0, 0.6)
                if xnb1 is None:
                    xnb1 = [ldbf(xnw[1, k]) for k in range(NT)]
                bu, ticks = job_m1(xnb1, n)
                hr, hi, cy = _scan_tile(bu[:, :128], bu[:, 128:], lambda i, n=n: tab(i, n), cy, NP)
                hs1.append(jnp.concatenate([hr, hi], axis=1).astype(BF16))
                carry.append(cy)
                place(ticks, 640, 256 + 830, [])
    with scope("wc"):
        wait(("c", 0))
        issue_fakes()
        if ipos[1] == 3:
            issue_kv0()
    dma_kv(1)
    dma_kv(2)
    with scope("a1_0m2"):
        flush(cprep_lumps(0))
        m2_part(hs0, rwin(xr_ref, 0), [cprep_lumps(k + 1) if k + 1 < NT else [] for k in range(NT)], True)
    with scope("w_x2kv0"):
        wait(*opts.get("w0", ()))
    with scope("a1_1m2"):
        m2_part(hs1, rwin(xr_ref, 1), [[]] * NT, False)
        put_carry(carry)
    late_issue = [lambda: dma_kv(3)]
    dma_x(("kv", 1), 4 * T, S)

    def a1_block(j):
        carry = get_carry()
        hs, carry = m1_part(carry, [], j % 2)
        put_carry(carry)
        if j + 1 < NB:
            s1 = split(s1a_lumps(xwin(j + 1), rwin(xr_ref, j + 1), (j + 1) % 2), 4)
            m2_part(hs, rwin(xr_ref, j), s1, True)
        else:
            force((NCH - 2) * NCH * NT)
            yc, tg = job_g(zwin(0))
            place(tg, 640, 160 + 830, [])
            s1 = split(s1b_lumps(yc, rwin(yk_ref, 0), rwin(xr_ref, 0), 0), 4)
            m2_part(hs, rwin(xr_ref, j), s1, False)

    dpos = opts.get("dpos", (2, 3, 4, 5))
    for j in range(2, NB):
        for q in range(NQ):
            if dpos[q] == j:
                with scope(f"dft{q}"):
                    wq = opts.get("wq", {0: (("kv", 0),), 1: (("kv", 1),), 2: (("kv", 2),), 3: (("kv", 3),)})
                    with scope(f"w_q{q}"):
                        wait(*wq[q])
                    if q in opts.get("extrabar", (("a1", 2), ("a1", 3), ("a1", 4), ("a1", 5))):
                        fake_barrier()
                    if late_issue:
                        late_issue.pop()()
                    ex = s1a_lumps(xwin(2), rwin(xr_ref, 2), 0) if q == 0 else ()
                    barrier(lambda q=q: dft_group(q * CQ, CQ, ex))
        if ("a1", j) in opts.get("extrabar", (("a1", 2), ("a1", 3), ("a1", 4), ("a1", 5))):
            fake_barrier()
        with scope(f"a1_{j}"):
            barrier(lambda j=j: a1_block(j))

    cur_util[0] = opts.get("util2", 0.55)
    for n in range(NT):
        carry_ref[2 * n] = jnp.zeros((8, 128), F32)
        carry_ref[2 * n + 1] = jnp.zeros((8, 128), F32)

    def a2_block(j):
        carry = get_carry()
        prev3 = s3_lumps(rwin(xr_ref, j - 1), rwin(yk_ref, j - 1), obwin(j - 1)) if j > 0 else []
        hs, carry = m1_part(carry, prev3, j % 2)
        put_carry(carry)
        if j + 1 < NB:
            force((NCH - 2 * (j + 2)) * NCH * NT)
            yc, tg = job_g(zwin(j + 1))
            place(tg, 640, 160 + 830, [])
            s1 = split(s1b_lumps(yc, rwin(yk_ref, j + 1), rwin(xr_ref, j + 1), (j + 1) % 2), 4)
        else:
            if j > 0:
                out_dma(j - 1)
            s1 = [[]] * NT
        m2_part(hs, rwin(xr_ref, j), s1, j + 1 == NB)

    for j in range(NB):
        if ("a2", j) in opts.get("extrabar", (("a1", 2), ("a1", 3), ("a1", 4), ("a1", 5))):
            fake_barrier()
        with scope(f"a2_{j}"):
            barrier(lambda j=j: a2_block(j))
        if 0 < j < NB - 1:
            out_dma(j - 1)
    with scope("tail"):
        flush(filler)
        del filler[:]
        l3 = s3_lumps(rwin(xr_ref, NB - 1), rwin(yk_ref, NB - 1), obwin(NB - 1))
        ng = opts.get("tailg", 4)
        per = len(l3) // ng
        rows_per = T // ng
        for i in range(ng):
            flush(l3[i * per:(i + 1) * per])
            for n in range(NT):
                r0 = (NB - 1) * T + i * rows_per
                pltpu.make_async_copy(ob.at[n, pl.ds(r0, rows_per)],
                                      o_hbm.at[pl.ds(r0, rows_per), pl.ds(128 * n, 128)], osems.at[0]).start()
    with scope("fin"):
        for n in range(NT):
            pltpu.make_async_copy(ob.at[n, 0:S], o_hbm.at[:, pl.ds(128 * n, 128)], osems.at[0]).wait()
    if opts.get("nofill"):
        print("JOBDUR", jobdur)
    if opts.get("verbose"):
        print("filler left", len(filler), sum(c for c, _ in filler))


def make(NP=4, **opts):
    fn_np, fp_np, gp_np = _dft_consts(NP)
    zero_np = np.concatenate([np.zeros((8, 128), np.int32), np.ones((8, 128), np.int32)])

    @jax.jit
    def fn(A_x, A_Lambda_re, A_Lambda_im, A_B_re, A_B_im, A_C_re, A_C_im, A_log_dt, A_Dskip,
           B_q, B_k, B_v, B_shift_k, B_ssm_k, B_ssm_D):
        del B_q
        args = (A_x.reshape(S, D), A_Lambda_re, A_Lambda_im, A_B_re, A_B_im, A_C_re, A_C_im,
                A_log_dt, A_Dskip, B_k.reshape(S, D), B_v.reshape(S, D), B_shift_k.T, B_ssm_k,
                B_ssm_D, jnp.asarray(fn_np, BF16), jnp.asarray(fp_np, BF16), jnp.asarray(gp_np, BF16),
                jnp.asarray(zero_np))
        hbm = pl.BlockSpec(memory_space=pltpu.HBM)
        vm = pl.BlockSpec(memory_space=pltpu.VMEM)
        out = pl.pallas_call(
            functools.partial(_kernel, NP=NP, opts=opts),
            out_shape=jax.ShapeDtypeStruct((S, D), F32),
            **({"grid": (1,)} if opts.get("opq_st") else {}),
            in_specs=[hbm] * 18,
            out_specs=hbm,
            scratch_shapes=[
                pltpu.VMEM((D,), BF16), pltpu.VMEM((D,), BF16), pltpu.VMEM((D,), BF16),
                pltpu.VMEM((D,), BF16), pltpu.VMEM((D,), BF16),
                pltpu.VMEM((4, D), BF16),
                pltpu.VMEM((2 * L, L), BF16), pltpu.VMEM((2 * L, L), BF16), pltpu.VMEM((L, 2 * L), BF16),
                pltpu.VMEM((16, 128), jnp.int32),
                pltpu.VMEM((NT, S + 16, 128), BF16),
                pltpu.VMEM((NT, S, 128), BF16),
                pltpu.VMEM((NT, S, 128), BF16),
                pltpu.VMEM((NCH, D, L), BF16),
                pltpu.VMEM((NT, D, 128), BF16),
                pltpu.VMEM((NT, D, 128), BF16),
                pltpu.VMEM((NT, D, 128), BF16),
                pltpu.VMEM((NT, D, 128), BF16),
                pltpu.VMEM((NT, 2, D, 128), BF16),
                pltpu.VMEM((2, NT, T, 128), BF16),
                pltpu.VMEM((18, 8, D), F32),
                pltpu.VMEM((NCH, 2 * L, D), F32),
                pltpu.VMEM((NCH, 2 * L, D), F32),
                pltpu.VMEM((NCH, 16, D), F32),
                pltpu.VMEM((NT, NCH * 2 * L, 128), BF16),
                pltpu.VMEM((S, D), F32),
                pltpu.VMEM((S + T, D), F32),
                pltpu.VMEM((NT, S, 128), F32),
                pltpu.VMEM((2 * NT, 8, 128), F32),
                pltpu.VMEM((4, NT, L, 128), BF16),
                pltpu.VMEM((16, 16, 128), jnp.int32),
                pltpu.SemaphoreType.DMA((NSEM,)),
                pltpu.SemaphoreType.DMA((1,)),
            ],
            compiler_params=pltpu.CompilerParams(vmem_limit_bytes=110 * 1024 * 1024,
                                                 **({"flags": opts["flags"]} if "flags" in opts else {})),
            name="ssm_fused",
        )(*args)
        return out.reshape(1, S, D)
    return fn


pallas_interleave_layers__ssm_conv_s5__ssm_conv_h3__prompt_kernel = make(
    dpos=(2, 3, 4, 4), extrabar=(("a1", 2), ("a1", 3), ("a1", 4)),
    wq={0: (("kv", 0),), 1: (("kv", 1),), 2: (("kv", 2), ("kv", 3)), 3: ()}, util=0.7, util2=0.62)
```
